```python
import jax
import jax.numpy as jnp

def _softmax(x, axis=-1):
    return jax.nn.softmax(x, axis=axis)

def _gelu(x):
    return jax.nn.gelu(x, approximate=True)

def _silu(x):
    return jax.nn.silu(x)

def _sigmoid(x):
    return jax.nn.sigmoid(x)

def _layernorm(x, axis=-1, eps=1e-05):
    m = jnp.mean(x, axis=axis, keepdims=True)
    v = jnp.var(x, axis=axis, keepdims=True)
    return (x - m) / jnp.sqrt(v + eps)

def _scatter_add(tgt, idx, src, axis=0):
    return tgt.at[idx].add(src)

def _segment_sum(src, seg, n):
    return jax.ops.segment_sum(src, seg, n)

class _Rng:

    def __init__(self, key):
        self._k = key

    def _next(self):
        self._k, sub = jax.random.split(self._k)
        return sub

    def normal(self, shape):
        return jax.random.normal(self._next(), shape, dtype=jnp.bfloat16)

    def randint(self, lo, hi, shape):
        return jax.random.randint(self._next(), shape, lo, hi, dtype=jnp.int32)

    def uniform(self, shape, lo=0.0, hi=1.0):
        return jax.random.uniform(self._next(), shape, jnp.bfloat16, lo, hi)

    def permutation(self, n):
        return jax.random.permutation(self._next(), n)
kernel_name = 'gated_mix__memory_aug_recurrent_mem_tr__sliding_local_dilated__prompt'

def setup_inputs():
    _rng = _Rng(jax.random.key(int.from_bytes(__import__("os").urandom(4), "little")))
    _w = lambda a: (lambda t: t.astype(jnp.bfloat16) if jnp.issubdtype(t.dtype, jnp.floating) else t)(jnp.asarray(a))

    def _A_setup():
        B, S, Dm = (1, 2048, 640)
        H, Dh = (32, 192)
        M, seg = (8, 32)
        seg = min(seg, S)
        S = S // seg * seg
        return {'x': _w((lambda *s: _rng.normal(s) * 0.05)(B, S, Dm)), 'mem0': _w((lambda *s: _rng.normal(s) * 0.05)(B, M, Dm)), 'Wq': _w((lambda *s: _rng.normal(s) * 0.05)(Dm, H, Dh) * Dm ** (-0.5)), 'Wk': _w((lambda *s: _rng.normal(s) * 0.05)(Dm, H, Dh) * Dm ** (-0.5)), 'Wv': _w((lambda *s: _rng.normal(s) * 0.05)(Dm, H, Dh) * Dm ** (-0.5)), 'Wo': _w((lambda *s: _rng.normal(s) * 0.05)(H, Dh, Dm) * (H * Dh) ** (-0.5)), 'seg_len': seg}
    _A_in = _A_setup()

    def _B_setup():
        B, S, D = (1, 2048, 640)
        return {'x': _w((lambda *s: _rng.normal(s) * 0.05)(B, S, D)), 'wqkv': _w((lambda *s: _rng.normal(s) * 0.05)(D, 3 * D)), 'wo': _w((lambda *s: _rng.normal(s) * 0.05)(D, D))}
    _B_in = _B_setup()
    return {'A_x': _A_in['x'], 'A_mem0': _A_in['mem0'], 'A_Wq': _A_in['Wq'], 'A_Wk': _A_in['Wk'], 'A_Wv': _A_in['Wv'], 'A_Wo': _A_in['Wo'], 'A_seg_len': _A_in['seg_len'], 'B_x': _B_in['x'], 'B_wqkv': _B_in['wqkv'], 'B_wo': _B_in['wo'], 'gate_w': _w((lambda *s: _rng.normal(s) * 0.05)(640))}

def reference(A_x, A_mem0, A_Wq, A_Wk, A_Wv, A_Wo, A_seg_len, B_x, B_wqkv, B_wo, gate_w):

    def _A_ref(x, mem0, Wq, Wk, Wv, Wo, seg_len):
        B, S, Dm = x.shape
        H, Dh = (Wq.shape[1], Wq.shape[2])
        M = mem0.shape[1]
        scale = Dh ** (-0.5)
        n_seg = S // seg_len
        L = M + seg_len
        idx = jnp.arange(L)
        mask = (idx[:, None] < M) | (idx[:, None] >= idx[None, :])
        mem = mem0
        outs = []
        for s in range(n_seg):
            xs = x[:, s * seg_len:(s + 1) * seg_len, :].copy()
            h = jnp.concatenate([mem, xs], axis=1)
            q = jnp.einsum('btd,dhe->bhte', h, Wq)
            k = jnp.einsum('btd,dhe->bhte', h, Wk)
            v = jnp.einsum('btd,dhe->bhte', h, Wv)
            scores = jnp.einsum('bhqe,bhke->bhqk', q, k) * scale
            scores = jnp.where(mask[None, None], scores, -1000000000.0)
            p = _softmax(scores, axis=-1)
            o = jnp.einsum('bhqk,bhke->bhqe', p, v)
            o = jnp.einsum('bhte,hed->btd', o, Wo)
            mem = o[:, :M, :].copy()
            outs.append(o[:, M:, :])
        return jnp.concatenate(outs, axis=1)

    def _B_ref(x, wqkv, wo):
        B, S, D = x.shape
        H = 32
        Dh = D // H
        W, dil = (8, 2)
        qkv = (lambda x, *d: x.transpose(*d))((x @ wqkv).reshape(B, S, 3, H, Dh), 2, 0, 3, 1, 4)
        q, k, v = (qkv[0], qkv[1], qkv[2])
        scale = Dh ** (-0.5)
        pos = jnp.arange(S)
        off = jnp.arange(W) * dil
        idx = pos[:, None] - off[None, :]
        mask = idx >= 0
        idx_c = jnp.where(mask, idx, 0).reshape(-1)
        kg = k[:, :, idx_c, :].reshape(B, H, S, W, Dh)
        vg = v[:, :, idx_c, :].reshape(B, H, S, W, Dh)
        logits = jnp.einsum('bhsd,bhswd->bhsw', q, kg) * scale
        logits = jnp.where(mask[None, None, :, :], logits, -1000000000.0)
        attn = _softmax(logits, axis=-1)
        o = jnp.einsum('bhsw,bhswd->bhsd', attn, vg)
        return (lambda x, *d: x.transpose(*d))(o, 0, 2, 1, 3).reshape(B, S, D) @ wo
    x = A_x
    g = _sigmoid((x * gate_w).sum(-1, keepdims=True))
    a = _A_ref(x, A_mem0, A_Wq, A_Wk, A_Wv, A_Wo, A_seg_len)
    b = _B_ref(x, B_wqkv, B_wo)
    return g * a + (1 - g) * b
```

```python
import functools

import jax
import jax.numpy as jnp
import jax.experimental.pallas as pl
import jax.experimental.pallas.tpu as pltpu

F32 = jnp.float32
BF16 = jnp.bfloat16

_NN = (((1,), (0,)), ((), ()))
_NT = (((1,), (1,)), ((), ()))

_B_HEADS = 32
_B_WIN = 8
_B_DIL = 2
_B_PAD = 16
_B_ROWS = 128


def _dot(a, b, dims=_NN):
    return jax.lax.dot_general(a, b, dims, preferred_element_type=F32)


def _kernel(x_hbm, mem0_ref, wqt_hbm, wkt_hbm, wvt_hbm, wo_hbm, bwqkv_hbm,
            bwo_hbm, gw_ref, out_hbm,
            x_v, wt_v, w_v, wo_v, bw_v, bwp_v, bwo_v, bwop_v, kv_v, b_v,
            mem_v, out_v, sem_in, sem_w, sem_out, *, seg, n_heads, dh):
    S, D = x_v.shape
    M = mem0_ref.shape[0]
    L = M + seg
    n_seg = S // seg
    pw = 2 * dh
    n_pairs = n_heads // 2
    bdh = D // _B_HEADS

    cp_bw = pltpu.make_async_copy(bwqkv_hbm, bw_v, sem_in.at[0])
    cp_x = pltpu.make_async_copy(x_hbm, x_v, sem_in.at[1])
    cp_bwo = pltpu.make_async_copy(bwo_hbm, bwo_v, sem_in.at[2])
    cp_wo = pltpu.make_async_copy(wo_hbm, wo_v, sem_in.at[3])

    def cp_w(t, p):
        src = (wqt_hbm, wkt_hbm, wvt_hbm)[t]
        return pltpu.make_async_copy(src.at[p], wt_v.at[p, t], sem_w.at[p, t])

    cp_bw.start()
    cp_x.start()
    cp_bwo.start()
    for p in range(n_pairs):
        for t in range(3):
            cp_w(t, p).start()
    cp_wo.start()

    ri = jax.lax.broadcasted_iota(jnp.int32, (D, D), 0)
    ci = jax.lax.broadcasted_iota(jnp.int32, (D, D), 1)
    perm = jnp.where(ri == (ci % _B_HEADS) * bdh + ci // _B_HEADS, 1.0, 0.0).astype(BF16)
    perm_t = jnp.where(ci == (ri % _B_HEADS) * bdh + ri // _B_HEADS, 1.0, 0.0).astype(BF16)
    kv_v[pl.ds(_B_ROWS, _B_PAD), :] = jnp.zeros((_B_PAD, 2 * D), F32)
    cp_bw.wait()
    for t in range(3):
        bwp_v[:, t * D:(t + 1) * D] = _dot(bw_v[:, t * D:(t + 1) * D], perm).astype(BF16)
    cp_bwo.wait()
    bwop_v[...] = _dot(perm_t, bwo_v[...]).astype(BF16)
    cp_x.wait()

    b_scale = bdh ** (-0.5)
    n_grp = D // 128

    def startup(i, carry):
        r0 = pl.multiple_of(i * _B_ROWS, _B_ROWS)
        xb = x_v[pl.ds(r0, _B_ROWS), :]
        q = _dot(xb, bwp_v[:, 0:D])
        kv_v[pl.ds(0, _B_PAD), :] = kv_v[pl.ds(_B_ROWS, _B_PAD), :]
        kv_v[pl.ds(_B_PAD, _B_ROWS), :] = _dot(xb, bwp_v[:, D:3 * D])
        pos = r0 + jax.lax.broadcasted_iota(jnp.int32, (_B_ROWS, 128), 0)
        logits = []
        for w in range(_B_WIN):
            kw = kv_v[pl.ds(_B_PAD - w * _B_DIL, _B_ROWS), 0:D]
            pr = q * kw
            acc = pr[:, 0:128]
            for g in range(1, n_grp):
                acc = acc + pr[:, g * 128:(g + 1) * 128]
            acc = acc + pltpu.roll(acc, 64, 1)
            acc = acc + pltpu.roll(acc, 32, 1)
            lg = acc * b_scale
            if w > 0:
                lg = jnp.where(pos >= w * _B_DIL, lg, -1e9)
            logits.append(lg)
        m = functools.reduce(jnp.maximum, logits)
        es = [jnp.exp(lg - m) for lg in logits]
        inv = 1.0 / functools.reduce(jnp.add, es)
        o = None
        for w in range(_B_WIN):
            vw = kv_v[pl.ds(_B_PAD - w * _B_DIL, _B_ROWS), D:2 * D]
            a = es[w] * inv
            t = jnp.concatenate([a] * n_grp, axis=1) * vw
            o = t if o is None else o + t
        b_v[pl.ds(r0, _B_ROWS), :] = _dot(o.astype(BF16), bwop_v[...])
        for t in range(3):
            cp_w(t, i).wait()
            w_v[i, :, t * pw:(t + 1) * pw] = wt_v[i, t].T
        return carry

    jax.lax.fori_loop(0, n_pairs, startup, 0)
    cp_wo.wait()

    a_scale = dh ** (-0.5)
    mem_v[...] = mem0_ref[...].astype(F32)

    def step(s, carry):
        r0 = pl.multiple_of(s * seg, seg)
        xs = x_v[pl.ds(r0, seg), :].astype(F32)
        h = jnp.concatenate([mem_v[...], xs], axis=0)

        row = jax.lax.broadcasted_iota(jnp.int32, (L, 2 * L), 0)
        col = jax.lax.broadcasted_iota(jnp.int32, (L, 2 * L), 1)
        first = col < L
        key = jnp.where(first, col, col - L)
        visible = (row < M) | (row >= key)
        lane = jax.lax.broadcasted_iota(jnp.int32, (L, 128), 1)
        lo = lane < (dh - 128)
        zero = jnp.zeros((L, 128), F32)

        def block_diag(a):
            mid = a[:, 128:256]
            top = jnp.concatenate([a[:, 0:128], jnp.where(lo, mid, 0.0), zero], axis=1)
            bot = jnp.concatenate([zero, jnp.where(lo, 0.0, mid), a[:, 256:384]], axis=1)
            return jnp.concatenate([top, bot], axis=0).astype(BF16)

        acc = None
        for p in range(n_pairs):
            qkv = _dot(h, w_v[p])
            q = qkv[:, 0:pw]
            sc = _dot(q, block_diag(qkv[:, pw:2 * pw]), _NT) * a_scale
            sc = jnp.where(visible, sc, -1e9)
            m0 = jnp.max(jnp.where(first, sc, -jnp.inf), axis=1, keepdims=True)
            m1 = jnp.max(jnp.where(first, -jnp.inf, sc), axis=1, keepdims=True)
            e = jnp.exp(sc - jnp.where(first, m0, m1))
            l0 = jnp.sum(jnp.where(first, e, 0.0), axis=1, keepdims=True)
            l1 = jnp.sum(jnp.where(first, 0.0, e), axis=1, keepdims=True)
            pr = e * jnp.where(first, 1.0 / l0, 1.0 / l1)
            o = _dot(pr, block_diag(qkv[:, 2 * pw:3 * pw]))
            t = _dot(o, wo_v[p])
            acc = t if acc is None else acc + t

        mem_v[...] = acc[0:M]
        g = jax.nn.sigmoid(jnp.sum(xs * gw_ref[...].astype(F32), axis=1, keepdims=True))
        res = g * acc[M:L] + (1.0 - g) * b_v[pl.ds(r0, seg), :]
        out_v[pl.ds(r0, seg), :] = res.astype(out_v.dtype)
        pltpu.make_async_copy(out_v.at[pl.ds(r0, seg)], out_hbm.at[pl.ds(r0, seg)],
                              sem_out.at[0]).start()
        return carry

    jax.lax.fori_loop(0, n_seg, step, 0)
    pltpu.make_async_copy(out_v, out_hbm, sem_out.at[0]).wait()


@functools.partial(jax.jit, static_argnames=("A_seg_len",))
def pallas_gated_mix__memory_aug_recurrent_mem_tr__sliding_local_dilated__prompt_kernel(
    A_x, A_mem0, A_Wq, A_Wk, A_Wv, A_Wo, A_seg_len, B_x, B_wqkv, B_wo, gate_w,
):
    del B_x
    _, S, D = A_x.shape
    M = A_mem0.shape[1]
    _, H, Dh = A_Wq.shape
    seg = int(A_seg_len)
    n_pairs = H // 2
    pw = 2 * Dh
    assert Dh == 192 and S == n_pairs * _B_ROWS and S % seg == 0 and D % 128 == 0

    def wt(w):
        return jnp.transpose(w, (1, 2, 0)).reshape(n_pairs, pw, D)

    hbm = pl.BlockSpec(memory_space=pl.ANY)
    vmem = pl.BlockSpec(memory_space=pltpu.VMEM)
    out = pl.pallas_call(
        functools.partial(_kernel, seg=seg, n_heads=H, dh=Dh),
        out_shape=jax.ShapeDtypeStruct((S, D), A_x.dtype),
        in_specs=[hbm, vmem, hbm, hbm, hbm, hbm, hbm, hbm, vmem],
        out_specs=hbm,
        scratch_shapes=[
            pltpu.VMEM((S, D), BF16),
            pltpu.VMEM((n_pairs, 3, pw, D), BF16),
            pltpu.VMEM((n_pairs, D, 3 * pw), BF16),
            pltpu.VMEM((n_pairs, pw, D), BF16),
            pltpu.VMEM((D, 3 * D), BF16),
            pltpu.VMEM((D, 3 * D), BF16),
            pltpu.VMEM((D, D), BF16),
            pltpu.VMEM((D, D), BF16),
            pltpu.VMEM((_B_ROWS + _B_PAD, 2 * D), F32),
            pltpu.VMEM((S, D), F32),
            pltpu.VMEM((M, D), F32),
            pltpu.VMEM((S, D), A_x.dtype),
            pltpu.SemaphoreType.DMA((4,)),
            pltpu.SemaphoreType.DMA((n_pairs, 3)),
            pltpu.SemaphoreType.DMA((1,)),
        ],
        compiler_params=pltpu.CompilerParams(vmem_limit_bytes=110 * 1024 * 1024),
    )(A_x.reshape(S, D), A_mem0.reshape(M, D), wt(A_Wq), wt(A_Wk), wt(A_Wv),
      A_Wo.reshape(n_pairs, pw, D), B_wqkv, B_wo, gate_w.reshape(1, D))
    return out.reshape(A_x.shape)
```

```python
import functools

import jax
import jax.numpy as jnp
import jax.experimental.pallas as pl
import jax.experimental.pallas.tpu as pltpu

F32 = jnp.float32
BF16 = jnp.bfloat16

_NN = (((1,), (0,)), ((), ()))
_NT = (((1,), (1,)), ((), ()))

_B_HEADS = 32
_B_WIN = 8
_B_DIL = 2
_B_PAD = 16
_B_CHUNK = 16
_B_ROWS = 128
_LAGS = (1, 2, 3, 4)


def _dot(a, b, dims=_NN):
    return jax.lax.dot_general(a, b, dims, preferred_element_type=F32)


def _kernel(x_hbm, mem0_ref, wqt_hbm, wkt_hbm, wvt_hbm, wo_hbm, bwqkv_hbm,
            bwo_hbm, gw_ref, out_hbm,
            x_v, wt_v, w_v, wo_v, bw_v, bwp_v, bwo_v, bwop_v, perm_v,
            q0_v, kv0_v, ob0_v, q1_v, kv1_v, ob1_v, sh_v, b_v,
            mem_v, out_v, sem_in, sem_w, sem_out, *, seg, n_heads, dh):
    S, D = x_v.shape
    M = mem0_ref.shape[0]
    L = M + seg
    n_seg = S // seg
    pw = 2 * dh
    n_pairs = n_heads // 2
    bdh = D // _B_HEADS

    cp_bw = pltpu.make_async_copy(bwqkv_hbm, bw_v, sem_in.at[0])
    cp_x = pltpu.make_async_copy(x_hbm, x_v, sem_in.at[1])
    cp_bwo = pltpu.make_async_copy(bwo_hbm, bwo_v, sem_in.at[2])
    cp_wo = pltpu.make_async_copy(wo_hbm, wo_v, sem_in.at[3])

    def cp_w(t, p):
        src = (wqt_hbm, wkt_hbm, wvt_hbm)[t]
        return pltpu.make_async_copy(src.at[p], wt_v.at[p, t], sem_w.at[p, t])

    cp_bw.start()
    cp_x.start()
    cp_bwo.start()

    ri = jax.lax.broadcasted_iota(jnp.int32, (D, D), 0)
    ci = jax.lax.broadcasted_iota(jnp.int32, (D, D), 1)
    perm_v[0] = jnp.where(ri == (ci % _B_HEADS) * bdh + ci // _B_HEADS, 1.0, 0.0).astype(BF16)
    perm_v[1] = jnp.where(ci == (ri % _B_HEADS) * bdh + ri // _B_HEADS, 1.0, 0.0).astype(BF16)
    cp_bw.wait()
    for p in range(n_pairs):
        for t in range(3):
            cp_w(t, p).start()
    cp_wo.start()
    for t in range(3):
        bwp_v[:, t * D:(t + 1) * D] = _dot(bw_v[:, t * D:(t + 1) * D], perm_v[0]).astype(BF16)
    cp_bwo.wait()
    bwop_v[...] = _dot(perm_v[1], bwo_v[...]).astype(BF16)
    cp_x.wait()

    b_scale = bdh ** (-0.5)
    n_grp = D // 128
    R, P = _B_ROWS, _B_PAD

    def b_proj(i, buf, prev):
        q_v, kv_v, _ = buf
        xb = x_v[pl.ds(pl.multiple_of(i * R, R), R), :]
        q_v[...] = _dot(xb, bwp_v[:, 0:D])
        kv_v[0:P, :] = jnp.zeros((P, 2 * D), F32) if prev is None else prev[1][R:R + P, :]
        kv_v[P:P + R, :] = _dot(xb, bwp_v[:, D:3 * D])

    def b_attn(buf, first_block):
        q_v, kv_v, ob_v = buf
        for j in range(1, 8 // _B_DIL):
            sh_v[j - 1] = kv_v[P - 8 - j * _B_DIL:P + R - j * _B_DIL, :]

        def shifted(w, r, c0):
            hi, j = divmod(w, 8 // _B_DIL)
            if j == 0:
                return kv_v[P - 8 * hi + r:P - 8 * hi + r + _B_CHUNK, c0:c0 + D]
            return sh_v[j - 1, 8 - 8 * hi + r:8 - 8 * hi + r + _B_CHUNK, c0:c0 + D]

        for r in range(0, R, _B_CHUNK):
            q = q_v[r:r + _B_CHUNK, :]
            logits = []
            for w in range(_B_WIN):
                pr = q * shifted(w, r, 0)
                acc = pr[:, 0:128]
                for g in range(1, n_grp):
                    acc = acc + pr[:, g * 128:(g + 1) * 128]
                acc = acc + pltpu.roll(acc, 64, 1)
                acc = acc + pltpu.roll(acc, 32, 1)
                lg = acc * b_scale
                if first_block and r < w * _B_DIL:
                    pos = r + jax.lax.broadcasted_iota(jnp.int32, lg.shape, 0)
                    lg = jnp.where(pos >= w * _B_DIL, lg, -1e9)
                logits.append(lg)
            m = functools.reduce(jnp.maximum, logits)
            es = [jnp.exp(lg - m) for lg in logits]
            inv = 1.0 / functools.reduce(jnp.add, es)
            o = None
            for w in range(_B_WIN):
                t = jnp.concatenate([es[w] * inv] * n_grp, axis=1) * shifted(w, r, D)
                o = t if o is None else o + t
            ob_v[r:r + _B_CHUNK, :] = o.astype(BF16)

    def b_out(i, buf):
        b_v[pl.ds(pl.multiple_of(i * R, R), R), :] = _dot(buf[2][...], bwop_v[...])

    def a_weights(i):
        for t in range(3):
            w_v[i, :, t * pw:(t + 1) * pw] = wt_v[i, t].T

    def startup(i, cur, oth, first=False, last=False):
        for t in range(3):
            cp_w(t, i).wait()
        if not first:
            b_out(i - 1, oth)
        if not last:
            b_proj(i + 1, oth, cur)
        b_attn(cur, first)
        a_weights(i)

    buf0, buf1 = (q0_v, kv0_v, ob0_v), (q1_v, kv1_v, ob1_v)
    b_proj(0, buf0, None)
    startup(0, buf0, buf1, first=True)

    def startup2(j, carry):
        startup(2 * j + 1, buf1, buf0)
        startup(2 * j + 2, buf0, buf1)
        return carry

    jax.lax.fori_loop(0, n_pairs // 2 - 1, startup2, 0)
    startup(n_pairs - 1, buf1, buf0, last=True)
    b_out(n_pairs - 1, buf1)
    cp_wo.wait()

    a_scale = dh ** (-0.5)
    mem_v[...] = mem0_ref[...].astype(F32)

    def step(s, carry):
        r0 = pl.multiple_of(s * seg, seg)
        xs = x_v[pl.ds(r0, seg), :].astype(F32)
        h = jnp.concatenate([mem_v[...], xs], axis=0)

        row = jax.lax.broadcasted_iota(jnp.int32, (L, 2 * L), 0)
        col = jax.lax.broadcasted_iota(jnp.int32, (L, 2 * L), 1)
        first = col < L
        key = jnp.where(first, col, col - L)
        visible = (row < M) | (row >= key)
        lane = jax.lax.broadcasted_iota(jnp.int32, (L, 128), 1)
        lo = lane < (dh - 128)
        zero = jnp.zeros((L, 128), F32)

        def block_diag(a):
            mid = a[:, 128:256]
            top = jnp.concatenate([a[:, 0:128], jnp.where(lo, mid, 0.0), zero], axis=1)
            bot = jnp.concatenate([zero, jnp.where(lo, 0.0, mid), a[:, 256:384]], axis=1)
            return jnp.concatenate([top, bot], axis=0).astype(BF16)

        def proj(p):
            return _dot(h, w_v[p])

        def scores(qkv):
            sc = _dot(qkv[:, 0:pw], block_diag(qkv[:, pw:2 * pw]), _NT) * a_scale
            return sc, block_diag(qkv[:, 2 * pw:3 * pw])

        def softmax(sc):
            sc = jnp.where(visible, sc, -1e9)
            m0 = jnp.max(jnp.where(first, sc, -jnp.inf), axis=1, keepdims=True)
            m1 = jnp.max(jnp.where(first, -jnp.inf, sc), axis=1, keepdims=True)
            e = jnp.exp(sc - jnp.where(first, m0, m1))
            l0 = jnp.sum(jnp.where(first, e, 0.0), axis=1, keepdims=True)
            l1 = jnp.sum(jnp.where(first, 0.0, e), axis=1, keepdims=True)
            return e * jnp.where(first, 1.0 / l0, 1.0 / l1)

        lag_s, lag_m, lag_v, lag_o = _LAGS
        qkv, sv, pr, o = {}, {}, {}, {}
        acc = None
        for i in range(n_pairs + lag_o):
            if i < n_pairs:
                qkv[i] = proj(i)
            if 0 <= i - lag_s < n_pairs:
                sv[i - lag_s] = scores(qkv.pop(i - lag_s))
            if 0 <= i - lag_m < n_pairs:
                pr[i - lag_m] = softmax(sv[i - lag_m][0])
            if 0 <= i - lag_v < n_pairs:
                o[i - lag_v] = _dot(pr.pop(i - lag_v), sv.pop(i - lag_v)[1])
            if 0 <= i - lag_o < n_pairs:
                t = _dot(o.pop(i - lag_o), wo_v[i - lag_o])
                acc = t if acc is None else acc + t

        mem_v[...] = acc[0:M]
        g = jax.nn.sigmoid(jnp.sum(xs * gw_ref[...].astype(F32), axis=1, keepdims=True))
        res = g * acc[M:L] + (1.0 - g) * b_v[pl.ds(r0, seg), :]
        out_v[pl.ds(r0, seg), :] = res.astype(out_v.dtype)
        pltpu.make_async_copy(out_v.at[pl.ds(r0, seg)], out_hbm.at[pl.ds(r0, seg)],
                              sem_out.at[0]).start()
        return carry

    jax.lax.fori_loop(0, n_seg, step, 0)
    pltpu.make_async_copy(out_v, out_hbm, sem_out.at[0]).wait()


@functools.partial(jax.jit, static_argnames=("A_seg_len",))
def pallas_gated_mix__memory_aug_recurrent_mem_tr__sliding_local_dilated__prompt_kernel(
    A_x, A_mem0, A_Wq, A_Wk, A_Wv, A_Wo, A_seg_len, B_x, B_wqkv, B_wo, gate_w,
):
    del B_x
    _, S, D = A_x.shape
    M = A_mem0.shape[1]
    _, H, Dh = A_Wq.shape
    seg = int(A_seg_len)
    n_pairs = H // 2
    pw = 2 * Dh
    assert Dh == 192 and S == n_pairs * _B_ROWS and S % seg == 0 and D % 128 == 0

    def wt(w):
        return jnp.transpose(w, (1, 2, 0)).reshape(n_pairs, pw, D)

    b_bufs = [pltpu.VMEM((_B_ROWS, D), F32), pltpu.VMEM((_B_ROWS + _B_PAD, 2 * D), F32),
              pltpu.VMEM((_B_ROWS, D), BF16)]
    hbm = pl.BlockSpec(memory_space=pl.ANY)
    vmem = pl.BlockSpec(memory_space=pltpu.VMEM)
    out = pl.pallas_call(
        functools.partial(_kernel, seg=seg, n_heads=H, dh=Dh),
        out_shape=jax.ShapeDtypeStruct((S, D), A_x.dtype),
        in_specs=[hbm, vmem, hbm, hbm, hbm, hbm, hbm, hbm, vmem],
        out_specs=hbm,
        scratch_shapes=[
            pltpu.VMEM((S, D), BF16),
            pltpu.VMEM((n_pairs, 3, pw, D), BF16),
            pltpu.VMEM((n_pairs, D, 3 * pw), BF16),
            pltpu.VMEM((n_pairs, pw, D), BF16),
            pltpu.VMEM((D, 3 * D), BF16),
            pltpu.VMEM((D, 3 * D), BF16),
            pltpu.VMEM((D, D), BF16),
            pltpu.VMEM((D, D), BF16),
            pltpu.VMEM((2, D, D), BF16),
            *b_bufs, *b_bufs,
            pltpu.VMEM((8 // _B_DIL - 1, _B_ROWS + 8, 2 * D), F32),
            pltpu.VMEM((S, D), F32),
            pltpu.VMEM((M, D), F32),
            pltpu.VMEM((S, D), A_x.dtype),
            pltpu.SemaphoreType.DMA((4,)),
            pltpu.SemaphoreType.DMA((n_pairs, 3)),
            pltpu.SemaphoreType.DMA((1,)),
        ],
        compiler_params=pltpu.CompilerParams(vmem_limit_bytes=110 * 1024 * 1024),
    )(A_x.reshape(S, D), A_mem0.reshape(M, D), wt(A_Wq), wt(A_Wk), wt(A_Wv),
      A_Wo.reshape(n_pairs, pw, D), B_wqkv, B_wo, gate_w.reshape(1, D))
    return out.reshape(A_x.shape)
```

```python
import functools

import jax
import jax.numpy as jnp
import jax.experimental.pallas as pl
import jax.experimental.pallas.tpu as pltpu

F32 = jnp.float32
BF16 = jnp.bfloat16
U32 = jnp.uint32

_NN = (((1,), (0,)), ((), ()))
_NT = (((1,), (1,)), ((), ()))

_B_HEADS = 32
_B_WIN = 8
_B_DIL = 2
_B_PAD = 16
_B_CHUNK = 16
_B_ROWS = 128
_LAGS = (1, 2, 3, 4)


def _dot(a, b, dims=_NN):
    return jax.lax.dot_general(a, b, dims, preferred_element_type=F32)


def _pack(a):
    return pltpu.bitcast(a, U32)


def _unpack(a):
    return pltpu.bitcast(a, BF16)


def _interleave(*streams):
    todo = [((k + 0.5) / len(st), n, fn) for n, st in enumerate(streams) for k, fn in enumerate(st)]
    for _, _, fn in sorted(todo, key=lambda e: e[:2]):
        fn()


def _kernel(x_hbm, mem0_ref, wqt_hbm, wkt_hbm, wvt_hbm, wo_hbm, bwqkv_hbm,
            bwo_hbm, gw_ref, out_hbm,
            x_v, wt_v, w_v, wo_v, bw_v, bwp_v, bwo_v, bwop_v, tmp_v,
            q0_v, kv0_v, ob0_v, q1_v, kv1_v, ob1_v, sh_v, b_v,
            mem_v, out_v, sem_in, sem_w, sem_out, *, seg, n_heads, dh):
    S, D = x_v.shape
    M = mem0_ref.shape[0]
    L = M + seg
    n_seg = S // seg
    pw = 2 * dh
    n_pairs = n_heads // 2
    bdh = D // _B_HEADS

    cp_bw = pltpu.make_async_copy(bwqkv_hbm, bw_v, sem_in.at[0])
    cp_x = pltpu.make_async_copy(x_hbm, x_v, sem_in.at[1])
    cp_bwo = pltpu.make_async_copy(bwo_hbm, bwo_v, sem_in.at[2])

    def cp_w(t, p):
        src = (wqt_hbm, wkt_hbm, wvt_hbm, wo_hbm)[t]
        return pltpu.make_async_copy(src.at[p], wt_v.at[p, t], sem_w.at[p, t])

    cp_bw.start()
    cp_x.start()
    cp_bwo.start()

    def permute_rows(dst_v, r0):
        for g in range(D // 128):
            for d in range(bdh):
                rows = tmp_v[g, pl.ds(d, _B_HEADS, stride=bdh), :]
                r = (r0 + d * _B_HEADS) // 2
                dst_v[r:r + _B_HEADS // 2, g * 128:(g + 1) * 128] = _pack(rows.astype(BF16))

    cp_bw.wait()
    for p in range(n_pairs):
        for t in range(4):
            cp_w(t, p).start()
    for t in range(3):
        for g in range(D // 128):
            tmp_v[g] = bw_v[g * 128:(g + 1) * 128, t * D:(t + 1) * D].T.astype(F32)
        permute_rows(bwp_v, t * D)
    cp_bwo.wait()
    for g in range(D // 128):
        tmp_v[g] = bwo_v[:, g * 128:(g + 1) * 128].astype(F32)
    permute_rows(bwop_v, 0)
    cp_x.wait()

    b_scale = bdh ** (-0.5)
    n_grp = D // 128
    R, P = _B_ROWS, _B_PAD

    def b_proj(i, buf, prev):
        q_v, kv_v, _ = buf

        def halo():
            kv_v[0:P, :] = jnp.zeros((P, 2 * D), F32) if prev is None else prev[1][R:R + P, :]

        xb = x_v[pl.ds(pl.multiple_of(i * R, R), R), :]

        def piece(c):
            y = _dot(xb, _unpack(bwp_v[c // 2:c // 2 + 64, :]), _NT)
            if c < D:
                q_v[:, c:c + 128] = y
            else:
                kv_v[P:P + R, c - D:c - D + 128] = y

        return [halo] + [functools.partial(piece, c) for c in range(0, 3 * D, 128)]

    def b_attn(buf, first_block):
        q_v, kv_v, ob_v = buf
        def shift(j):
            sh_v[j - 1] = kv_v[P - 8 - j * _B_DIL:P + R - j * _B_DIL, :]

        def shifted(w, r, c0):
            hi, j = divmod(w, 8 // _B_DIL)
            if j == 0:
                return kv_v[P - 8 * hi + r:P - 8 * hi + r + _B_CHUNK, c0:c0 + D]
            return sh_v[j - 1, 8 - 8 * hi + r:8 - 8 * hi + r + _B_CHUNK, c0:c0 + D]

        def chunk(r):
            q = q_v[r:r + _B_CHUNK, :]
            logits = []
            for w in range(_B_WIN):
                pr = q * shifted(w, r, 0)
                acc = pr[:, 0:128]
                for g in range(1, n_grp):
                    acc = acc + pr[:, g * 128:(g + 1) * 128]
                acc = acc + pltpu.roll(acc, 64, 1)
                acc = acc + pltpu.roll(acc, 32, 1)
                lg = acc * b_scale
                if first_block and r < w * _B_DIL:
                    pos = r + jax.lax.broadcasted_iota(jnp.int32, lg.shape, 0)
                    lg = jnp.where(pos >= w * _B_DIL, lg, -1e9)
                logits.append(lg)
            m = functools.reduce(jnp.maximum, logits)
            es = [jnp.exp(lg - m) for lg in logits]
            inv = 1.0 / functools.reduce(jnp.add, es)
            o = None
            for w in range(_B_WIN):
                t = jnp.concatenate([es[w] * inv] * n_grp, axis=1) * shifted(w, r, D)
                o = t if o is None else o + t
            ob_v[r // 2:(r + _B_CHUNK) // 2, :] = _pack(o.astype(BF16))

        return ([functools.partial(shift, j) for j in range(1, 8 // _B_DIL)]
                + [functools.partial(chunk, r) for r in range(0, R, _B_CHUNK)])

    def b_out(i, buf):
        def piece(c):
            b_v[pl.ds(pl.multiple_of(i * R, R), R), c:c + 128] = _dot(
                _unpack(buf[2][...]), _unpack(bwop_v[:, c:c + 128]))

        return [functools.partial(piece, c) for c in range(0, D, 128)]

    def a_weights(i):
        def piece(t, c):
            if t < 3:
                w_v[i, :, t * pw + c:t * pw + c + 128] = _pack(wt_v[i, t, c:c + 128, :].T)
            else:
                wo_v[i, c // 2:c // 2 + 64, :] = _pack(wt_v[i, t, c:c + 128, :])

        return [functools.partial(piece, t, c) for t in range(4) for c in range(0, pw, 128)]

    def startup(i, cur, oth, first=False, last=False):
        for t in range(4):
            cp_w(t, i).wait()
        mm = ([] if first else b_out(i - 1, oth)) + ([] if last else b_proj(i + 1, oth, cur))
        k = len(mm) * 2 // 3
        _interleave(mm[:k], b_attn(cur, first))
        _interleave(mm[k:], a_weights(i))

    buf0, buf1 = (q0_v, kv0_v, ob0_v), (q1_v, kv1_v, ob1_v)
    _interleave(b_proj(0, buf0, None))
    startup(0, buf0, buf1, first=True)

    def startup2(j, carry):
        startup(2 * j + 1, buf1, buf0)
        startup(2 * j + 2, buf0, buf1)
        return carry

    jax.lax.fori_loop(0, n_pairs // 2 - 1, startup2, 0)
    startup(n_pairs - 1, buf1, buf0, last=True)
    _interleave(b_out(n_pairs - 1, buf1))

    a_scale = dh ** (-0.5)
    mem_v[...] = mem0_ref[...].astype(F32)

    def step(s, carry):
        r0 = pl.multiple_of(s * seg, seg)
        xs = x_v[pl.ds(r0, seg), :].astype(F32)
        h = jnp.concatenate([mem_v[...], xs], axis=0)

        row = jax.lax.broadcasted_iota(jnp.int32, (L, 2 * L), 0)
        col = jax.lax.broadcasted_iota(jnp.int32, (L, 2 * L), 1)
        first = col < L
        key = jnp.where(first, col, col - L)
        visible = (row < M) | (row >= key)
        lane = jax.lax.broadcasted_iota(jnp.int32, (L, 128), 1)
        lo = lane < (dh - 128)
        zero = jnp.zeros((L, 128), F32)

        def block_diag(a):
            mid = a[:, 128:256]
            top = jnp.concatenate([a[:, 0:128], jnp.where(lo, mid, 0.0), zero], axis=1)
            bot = jnp.concatenate([zero, jnp.where(lo, 0.0, mid), a[:, 256:384]], axis=1)
            return jnp.concatenate([top, bot], axis=0).astype(BF16)

        def proj(p):
            return _dot(h, _unpack(w_v[p]))

        def scores(qkv):
            sc = _dot(qkv[:, 0:pw], block_diag(qkv[:, pw:2 * pw]), _NT) * a_scale
            return sc, block_diag(qkv[:, 2 * pw:3 * pw])

        def softmax(sc):
            sc = jnp.where(visible, sc, -1e9)
            m0 = jnp.max(jnp.where(first, sc, -jnp.inf), axis=1, keepdims=True)
            m1 = jnp.max(jnp.where(first, -jnp.inf, sc), axis=1, keepdims=True)
            e = jnp.exp(sc - jnp.where(first, m0, m1))
            l0 = jnp.sum(jnp.where(first, e, 0.0), axis=1, keepdims=True)
            l1 = jnp.sum(jnp.where(first, 0.0, e), axis=1, keepdims=True)
            return e * jnp.where(first, 1.0 / l0, 1.0 / l1)

        lag_s, lag_m, lag_v, lag_o = _LAGS
        qkv, sv, pr, o = {}, {}, {}, {}
        acc = None
        for i in range(n_pairs + lag_o):
            if i < n_pairs:
                qkv[i] = proj(i)
            if 0 <= i - lag_s < n_pairs:
                sv[i - lag_s] = scores(qkv.pop(i - lag_s))
            if 0 <= i - lag_m < n_pairs:
                pr[i - lag_m] = softmax(sv[i - lag_m][0])
            if 0 <= i - lag_v < n_pairs:
                o[i - lag_v] = _dot(pr.pop(i - lag_v), sv.pop(i - lag_v)[1])
            if 0 <= i - lag_o < n_pairs:
                t = _dot(o.pop(i - lag_o), _unpack(wo_v[i - lag_o]))
                acc = t if acc is None else acc + t

        mem_v[...] = acc[0:M]
        g = jax.nn.sigmoid(jnp.sum(xs * gw_ref[...].astype(F32), axis=1, keepdims=True))
        res = g * acc[M:L] + (1.0 - g) * b_v[pl.ds(r0, seg), :]
        out_v[pl.ds(r0, seg), :] = res.astype(out_v.dtype)
        pltpu.make_async_copy(out_v.at[pl.ds(r0, seg)], out_hbm.at[pl.ds(r0, seg)],
                              sem_out.at[0]).start()
        return carry

    jax.lax.fori_loop(0, n_seg, step, 0)
    pltpu.make_async_copy(out_v, out_hbm, sem_out.at[0]).wait()


@functools.partial(jax.jit, static_argnames=("A_seg_len",))
def pallas_gated_mix__memory_aug_recurrent_mem_tr__sliding_local_dilated__prompt_kernel(
    A_x, A_mem0, A_Wq, A_Wk, A_Wv, A_Wo, A_seg_len, B_x, B_wqkv, B_wo, gate_w,
):
    del B_x
    _, S, D = A_x.shape
    M = A_mem0.shape[1]
    _, H, Dh = A_Wq.shape
    seg = int(A_seg_len)
    n_pairs = H // 2
    pw = 2 * Dh
    assert Dh == 192 and S == n_pairs * _B_ROWS and S % seg == 0 and D % 128 == 0

    def wt(w):
        return jnp.transpose(w, (1, 2, 0)).reshape(n_pairs, pw, D)

    b_bufs = [pltpu.VMEM((_B_ROWS, D), F32), pltpu.VMEM((_B_ROWS + _B_PAD, 2 * D), F32),
              pltpu.VMEM((_B_ROWS // 2, D), U32)]
    hbm = pl.BlockSpec(memory_space=pl.ANY)
    vmem = pl.BlockSpec(memory_space=pltpu.VMEM)
    out = pl.pallas_call(
        functools.partial(_kernel, seg=seg, n_heads=H, dh=Dh),
        out_shape=jax.ShapeDtypeStruct((S, D), A_x.dtype),
        in_specs=[hbm, vmem, hbm, hbm, hbm, hbm, hbm, hbm, vmem],
        out_specs=hbm,
        scratch_shapes=[
            pltpu.VMEM((S, D), BF16),
            pltpu.VMEM((n_pairs, 4, pw, D), BF16),
            pltpu.VMEM((n_pairs, D // 2, 3 * pw), U32),
            pltpu.VMEM((n_pairs, pw // 2, D), U32),
            pltpu.VMEM((D, 3 * D), BF16),
            pltpu.VMEM((3 * D // 2, D), U32),
            pltpu.VMEM((D, D), BF16),
            pltpu.VMEM((D // 2, D), U32),
            pltpu.VMEM((D // 128, D, 128), F32),
            *b_bufs, *b_bufs,
            pltpu.VMEM((8 // _B_DIL - 1, _B_ROWS + 8, 2 * D), F32),
            pltpu.VMEM((S, D), F32),
            pltpu.VMEM((M, D), F32),
            pltpu.VMEM((S, D), A_x.dtype),
            pltpu.SemaphoreType.DMA((3,)),
            pltpu.SemaphoreType.DMA((n_pairs, 4)),
            pltpu.SemaphoreType.DMA((1,)),
        ],
        compiler_params=pltpu.CompilerParams(vmem_limit_bytes=110 * 1024 * 1024),
    )(A_x.reshape(S, D), A_mem0.reshape(M, D), wt(A_Wq), wt(A_Wk), wt(A_Wv),
      A_Wo.reshape(n_pairs, pw, D), B_wqkv, B_wo, gate_w.reshape(1, D))
    return out.reshape(A_x.shape)
```

```python
import functools

import jax
import jax.numpy as jnp
import jax.experimental.pallas as pl
import jax.experimental.pallas.tpu as pltpu

F32 = jnp.float32
BF16 = jnp.bfloat16
U32 = jnp.uint32

_NN = (((1,), (0,)), ((), ()))
_NT = (((1,), (1,)), ((), ()))

_B_HEADS = 32
_B_WIN = 8
_B_DIL = 2
_B_PAD = 16
_B_CHUNK = 16
_B_ROWS = 128
_LAGS = (1, 2, 3, 4)


def _dot(a, b, dims=_NN):
    return jax.lax.dot_general(a, b, dims, preferred_element_type=F32)


def _pack(a):
    return pltpu.bitcast(a, U32)


def _unpack(a):
    return pltpu.bitcast(a, BF16)


def _interleave(*streams):
    todo = [((k + 0.5) / len(st), n, fn) for n, st in enumerate(streams) for k, fn in enumerate(st)]
    for _, _, fn in sorted(todo, key=lambda e: e[:2]):
        fn()


def _kernel(x_hbm, mem0_ref, wqt_hbm, wkt_hbm, wvt_hbm, wo_hbm, bwqkv_hbm,
            bwo_hbm, gw_ref, out_hbm,
            x_v, wt_v, w_v, wo_v, bw_v, bwp_v, bwo_v, bwop_v, tmp_v, same_head_v,
            q0_v, kv0_v, ob0_v, q1_v, kv1_v, ob1_v, b_v,
            mem_v, out_v, sem_in, sem_w, sem_out, *, seg, n_heads, dh):
    S, D = x_v.shape
    M = mem0_ref.shape[0]
    L = M + seg
    n_seg = S // seg
    pw = 2 * dh
    n_pairs = n_heads // 2
    bdh = D // _B_HEADS

    cp_bw = pltpu.make_async_copy(bwqkv_hbm, bw_v, sem_in.at[0])
    cp_x = pltpu.make_async_copy(x_hbm, x_v, sem_in.at[1])
    cp_bwo = pltpu.make_async_copy(bwo_hbm, bwo_v, sem_in.at[2])

    def cp_w(t, p):
        src = (wqt_hbm, wkt_hbm, wvt_hbm, wo_hbm)[t]
        return pltpu.make_async_copy(src.at[p], wt_v.at[p, t], sem_w.at[p, t])

    cp_bw.start()
    cp_x.start()
    cp_bwo.start()

    def permute_rows(dst_v, r0):
        for g in range(D // 128):
            for d in range(bdh):
                rows = tmp_v[g, pl.ds(d, _B_HEADS, stride=bdh), :]
                r = (r0 + d * _B_HEADS) // 2
                dst_v[r:r + _B_HEADS // 2, g * 128:(g + 1) * 128] = _pack(rows.astype(BF16))

    ri = jax.lax.broadcasted_iota(jnp.int32, (128, 128), 0)
    ci = jax.lax.broadcasted_iota(jnp.int32, (128, 128), 1)
    same_head_v[...] = _pack(jnp.where(ri % _B_HEADS == ci % _B_HEADS, 1.0, 0.0).astype(BF16))
    cp_bw.wait()
    for p in range(n_pairs):
        for t in range(4):
            cp_w(t, p).start()
    for t in range(3):
        for g in range(D // 128):
            tmp_v[g] = bw_v[g * 128:(g + 1) * 128, t * D:(t + 1) * D].T.astype(F32)
        permute_rows(bwp_v, t * D)
    cp_bwo.wait()
    for g in range(D // 128):
        tmp_v[g] = bwo_v[:, g * 128:(g + 1) * 128].astype(F32)
    permute_rows(bwop_v, 0)
    cp_x.wait()

    b_scale = bdh ** (-0.5)
    n_grp = D // 128
    R, P = _B_ROWS, _B_PAD

    def b_proj(i, buf, prev):
        q_v, kv_v, _ = buf
        xb = x_v[pl.ds(pl.multiple_of(i * R, R), R), :]

        def piece(c):
            y = _dot(xb, _unpack(bwp_v[c // 2:c // 2 + 64, :]), _NT)
            if c < D:
                q_v[:, c:c + 128] = y
                return
            cols = slice(c - D, c - D + 128)
            halo = jnp.zeros((P, 128), F32) if prev is None else prev[1][0, R - 8:R + 8, cols]
            y = jnp.concatenate([halo, y], axis=0)
            for j in range(8 // _B_DIL):
                kv_v[j, :, cols] = y[P - 8 - j * _B_DIL:P + R - j * _B_DIL]

        return [functools.partial(piece, c) for c in range(0, 3 * D, 128)]

    def b_attn(buf, first_block):
        q_v, kv_v, ob_v = buf

        def shifted(w, r, c0):
            hi, j = divmod(w, 8 // _B_DIL)
            return kv_v[j, 8 - 8 * hi + r:8 - 8 * hi + r + _B_CHUNK, c0:c0 + D]

        def chunk(r):
            q = q_v[r:r + _B_CHUNK, :]
            part = []
            for w in range(_B_WIN):
                pr = q * shifted(w, r, 0)
                acc = pr[:, 0:128]
                for g in range(1, n_grp):
                    acc = acc + pr[:, g * 128:(g + 1) * 128]
                part.append(acc)
            full = _dot(jnp.concatenate(part, axis=0), _unpack(same_head_v[...])) * b_scale
            logits = []
            for w in range(_B_WIN):
                lg = full[w * _B_CHUNK:(w + 1) * _B_CHUNK]
                if first_block and r < w * _B_DIL:
                    pos = r + jax.lax.broadcasted_iota(jnp.int32, lg.shape, 0)
                    lg = jnp.where(pos >= w * _B_DIL, lg, -1e9)
                logits.append(lg)
            m = functools.reduce(jnp.maximum, logits)
            es = [jnp.exp(lg - m) for lg in logits]
            inv = 1.0 / functools.reduce(jnp.add, es)
            o = None
            for w in range(_B_WIN):
                t = jnp.concatenate([es[w] * inv] * n_grp, axis=1) * shifted(w, r, D)
                o = t if o is None else o + t
            ob_v[r // 2:(r + _B_CHUNK) // 2, :] = _pack(o.astype(BF16))

        return [functools.partial(chunk, r) for r in range(0, R, _B_CHUNK)]

    def b_out(i, buf):
        def piece(c):
            b_v[pl.ds(pl.multiple_of(i * R, R), R), c:c + 128] = _dot(
                _unpack(buf[2][...]), _unpack(bwop_v[:, c:c + 128]))

        return [functools.partial(piece, c) for c in range(0, D, 128)]

    def a_weights(i):
        def piece(t, c):
            if t < 3:
                w_v[i, :, t * pw + c:t * pw + c + 128] = _pack(wt_v[i, t, c:c + 128, :].T)
            else:
                wo_v[i, c // 2:c // 2 + 64, :] = _pack(wt_v[i, t, c:c + 128, :])

        return [functools.partial(piece, t, c) for t in range(4) for c in range(0, pw, 128)]

    def startup(i, cur, oth, first=False, last=False):
        for t in range(4):
            cp_w(t, i).wait()
        mm = ([] if first else b_out(i - 1, oth)) + ([] if last else b_proj(i + 1, oth, cur))
        k = len(mm) * 2 // 3
        _interleave(mm[:k], b_attn(cur, first))
        _interleave(mm[k:], a_weights(i))

    buf0, buf1 = (q0_v, kv0_v, ob0_v), (q1_v, kv1_v, ob1_v)
    _interleave(b_proj(0, buf0, None))
    startup(0, buf0, buf1, first=True)

    def startup2(j, carry):
        startup(2 * j + 1, buf1, buf0)
        startup(2 * j + 2, buf0, buf1)
        return carry

    jax.lax.fori_loop(0, n_pairs // 2 - 1, startup2, 0)
    startup(n_pairs - 1, buf1, buf0, last=True)
    _interleave(b_out(n_pairs - 1, buf1))

    a_scale = dh ** (-0.5)
    mem_v[...] = mem0_ref[...].astype(F32)

    def step(s, carry):
        r0 = pl.multiple_of(s * seg, seg)
        xs = x_v[pl.ds(r0, seg), :].astype(F32)
        h = jnp.concatenate([mem_v[...], xs], axis=0)

        row = jax.lax.broadcasted_iota(jnp.int32, (L, 2 * L), 0)
        col = jax.lax.broadcasted_iota(jnp.int32, (L, 2 * L), 1)
        first = col < L
        key = jnp.where(first, col, col - L)
        visible = (row < M) | (row >= key)
        lane = jax.lax.broadcasted_iota(jnp.int32, (L, 128), 1)
        lo = lane < (dh - 128)
        zero = jnp.zeros((L, 128), F32)

        def block_diag(a):
            mid = a[:, 128:256]
            top = jnp.concatenate([a[:, 0:128], jnp.where(lo, mid, 0.0), zero], axis=1)
            bot = jnp.concatenate([zero, jnp.where(lo, 0.0, mid), a[:, 256:384]], axis=1)
            return jnp.concatenate([top, bot], axis=0).astype(BF16)

        def proj(p):
            return _dot(h, _unpack(w_v[p]))

        def scores(qkv):
            sc = _dot(qkv[:, 0:pw], block_diag(qkv[:, pw:2 * pw]), _NT) * a_scale
            return sc, block_diag(qkv[:, 2 * pw:3 * pw])

        def softmax(sc):
            sc = jnp.where(visible, sc, -1e9)
            m0 = jnp.max(jnp.where(first, sc, -jnp.inf), axis=1, keepdims=True)
            m1 = jnp.max(jnp.where(first, -jnp.inf, sc), axis=1, keepdims=True)
            e = jnp.exp(sc - jnp.where(first, m0, m1))
            l0 = jnp.sum(jnp.where(first, e, 0.0), axis=1, keepdims=True)
            l1 = jnp.sum(jnp.where(first, 0.0, e), axis=1, keepdims=True)
            return e * jnp.where(first, 1.0 / l0, 1.0 / l1)

        lag_s, lag_m, lag_v, lag_o = _LAGS
        qkv, sv, pr, o = {}, {}, {}, {}
        acc = None
        for i in range(n_pairs + lag_o):
            if i < n_pairs:
                qkv[i] = proj(i)
            if 0 <= i - lag_s < n_pairs:
                sv[i - lag_s] = scores(qkv.pop(i - lag_s))
            if 0 <= i - lag_m < n_pairs:
                pr[i - lag_m] = softmax(sv[i - lag_m][0])
            if 0 <= i - lag_v < n_pairs:
                o[i - lag_v] = _dot(pr.pop(i - lag_v), sv.pop(i - lag_v)[1])
            if 0 <= i - lag_o < n_pairs:
                t = _dot(o.pop(i - lag_o), _unpack(wo_v[i - lag_o]))
                acc = t if acc is None else acc + t

        mem_v[...] = acc[0:M]
        g = jax.nn.sigmoid(jnp.sum(xs * gw_ref[...].astype(F32), axis=1, keepdims=True))
        res = g * acc[M:L] + (1.0 - g) * b_v[pl.ds(r0, seg), :]
        out_v[pl.ds(r0, seg), :] = res.astype(out_v.dtype)
        pltpu.make_async_copy(out_v.at[pl.ds(r0, seg)], out_hbm.at[pl.ds(r0, seg)],
                              sem_out.at[0]).start()
        return carry

    jax.lax.fori_loop(0, n_seg, step, 0)
    pltpu.make_async_copy(out_v, out_hbm, sem_out.at[0]).wait()


@functools.partial(jax.jit, static_argnames=("A_seg_len",))
def pallas_gated_mix__memory_aug_recurrent_mem_tr__sliding_local_dilated__prompt_kernel(
    A_x, A_mem0, A_Wq, A_Wk, A_Wv, A_Wo, A_seg_len, B_x, B_wqkv, B_wo, gate_w,
):
    del B_x
    _, S, D = A_x.shape
    M = A_mem0.shape[1]
    _, H, Dh = A_Wq.shape
    seg = int(A_seg_len)
    n_pairs = H // 2
    pw = 2 * Dh
    assert Dh == 192 and S == n_pairs * _B_ROWS and S % seg == 0 and D % 128 == 0

    def wt(w):
        return jnp.transpose(w, (1, 2, 0)).reshape(n_pairs, pw, D)

    b_bufs = [pltpu.VMEM((_B_ROWS, D), F32),
              pltpu.VMEM((8 // _B_DIL, _B_ROWS + 8, 2 * D), F32),
              pltpu.VMEM((_B_ROWS // 2, D), U32)]
    hbm = pl.BlockSpec(memory_space=pl.ANY)
    vmem = pl.BlockSpec(memory_space=pltpu.VMEM)
    out = pl.pallas_call(
        functools.partial(_kernel, seg=seg, n_heads=H, dh=Dh),
        out_shape=jax.ShapeDtypeStruct((S, D), A_x.dtype),
        in_specs=[hbm, vmem, hbm, hbm, hbm, hbm, hbm, hbm, vmem],
        out_specs=hbm,
        scratch_shapes=[
            pltpu.VMEM((S, D), BF16),
            pltpu.VMEM((n_pairs, 4, pw, D), BF16),
            pltpu.VMEM((n_pairs, D // 2, 3 * pw), U32),
            pltpu.VMEM((n_pairs, pw // 2, D), U32),
            pltpu.VMEM((D, 3 * D), BF16),
            pltpu.VMEM((3 * D // 2, D), U32),
            pltpu.VMEM((D, D), BF16),
            pltpu.VMEM((D // 2, D), U32),
            pltpu.VMEM((D // 128, D, 128), F32),
            pltpu.VMEM((64, 128), U32),
            *b_bufs, *b_bufs,
            pltpu.VMEM((S, D), F32),
            pltpu.VMEM((M, D), F32),
            pltpu.VMEM((S, D), A_x.dtype),
            pltpu.SemaphoreType.DMA((3,)),
            pltpu.SemaphoreType.DMA((n_pairs, 4)),
            pltpu.SemaphoreType.DMA((1,)),
        ],
        compiler_params=pltpu.CompilerParams(vmem_limit_bytes=110 * 1024 * 1024),
    )(A_x.reshape(S, D), A_mem0.reshape(M, D), wt(A_Wq), wt(A_Wk), wt(A_Wv),
      A_Wo.reshape(n_pairs, pw, D), B_wqkv, B_wo, gate_w.reshape(1, D))
    return out.reshape(A_x.shape)
```

```python
import functools

import jax
import jax.numpy as jnp
import jax.experimental.pallas as pl
import jax.experimental.pallas.tpu as pltpu

F32 = jnp.float32
BF16 = jnp.bfloat16
U32 = jnp.uint32

_NN = (((1,), (0,)), ((), ()))
_NT = (((1,), (1,)), ((), ()))

_B_HEADS = 32
_B_WIN = 8
_B_DIL = 2
_B_PAD = 16
_B_CHUNK = 16
_B_ROWS = 128
_LAGS = (1, 2, 4, 6)
_UNROLL = 3


def _dot(a, b, dims=_NN):
    return jax.lax.dot_general(a, b, dims, preferred_element_type=F32)


def _pack(a):
    return pltpu.bitcast(a, U32)


def _unpack(a):
    return pltpu.bitcast(a, BF16)


def _interleave(*streams):
    todo = [((k + 0.5) / len(st), n, fn) for n, st in enumerate(streams) for k, fn in enumerate(st)]
    for _, _, fn in sorted(todo, key=lambda e: e[:2]):
        fn()


def _kernel(x_hbm, mem0_ref, wqt_hbm, wkt_hbm, wvt_hbm, wo_hbm, bwqkv_hbm,
            bwo_hbm, gw_ref, out_hbm,
            x_v, wt_v, w_v, wo_v, bw_v, bwp_v, bwo_v, bwop_v, tmp_v, same_head_v,
            q0_v, kv0_v, ob0_v, q1_v, kv1_v, ob1_v, b_v,
            mem_v, acc_v, out_v, sem_in, sem_w, sem_out, *, seg, n_heads, dh):
    S, D = x_v.shape
    M = mem0_ref.shape[0]
    L = M + seg
    n_seg = S // seg
    pw = 2 * dh
    n_pairs = n_heads // 2
    bdh = D // _B_HEADS

    cp_bw = pltpu.make_async_copy(bwqkv_hbm, bw_v, sem_in.at[0])
    x_head, x_tail = pl.ds(0, 2 * _B_ROWS), pl.ds(2 * _B_ROWS, S - 2 * _B_ROWS)
    cp_x0 = pltpu.make_async_copy(x_hbm.at[x_head], x_v.at[x_head], sem_in.at[1])
    cp_x1 = pltpu.make_async_copy(x_hbm.at[x_tail], x_v.at[x_tail], sem_in.at[3])
    cp_bwo = pltpu.make_async_copy(bwo_hbm, bwo_v, sem_in.at[2])

    def cp_w(t, p):
        src = (wqt_hbm, wkt_hbm, wvt_hbm, wo_hbm)[t]
        return pltpu.make_async_copy(src.at[p], wt_v.at[p, t], sem_w.at[p, t])

    cp_bw.start()
    cp_x0.start()
    cp_bwo.start()
    cp_x1.start()

    def permute_rows(dst_v, r0):
        for g in range(D // 128):
            for d in range(bdh):
                rows = tmp_v[g, pl.ds(d, _B_HEADS, stride=bdh), :]
                r = (r0 + d * _B_HEADS) // 2
                dst_v[r:r + _B_HEADS // 2, g * 128:(g + 1) * 128] = _pack(rows.astype(BF16))

    ri = jax.lax.broadcasted_iota(jnp.int32, (128, 128), 0)
    ci = jax.lax.broadcasted_iota(jnp.int32, (128, 128), 1)
    same_head_v[...] = _pack(jnp.where(ri % _B_HEADS == ci % _B_HEADS, 1.0, 0.0).astype(BF16))
    cp_bw.wait()
    for p in range(n_pairs):
        for t in range(4):
            cp_w(t, p).start()
    for t in range(3):
        for g in range(D // 128):
            tmp_v[g] = bw_v[g * 128:(g + 1) * 128, t * D:(t + 1) * D].T.astype(F32)
        permute_rows(bwp_v, t * D)

    b_scale = bdh ** (-0.5)
    n_grp = D // 128
    R, P = _B_ROWS, _B_PAD

    def b_proj(i, buf, prev):
        q_v, kv_v, _ = buf
        xb = x_v[pl.ds(pl.multiple_of(i * R, R), R), :]

        def piece(c):
            y = _dot(xb, _unpack(bwp_v[c // 2:c // 2 + 64, :]), _NT)
            if c < D:
                q_v[:, c:c + 128] = y
                return
            cols = slice(c - D, c - D + 128)
            halo = jnp.zeros((P, 128), F32) if prev is None else prev[1][0, R - 8:R + 8, cols]
            y = jnp.concatenate([halo, y], axis=0)
            for j in range(8 // _B_DIL):
                kv_v[j, :, cols] = y[P - 8 - j * _B_DIL:P + R - j * _B_DIL]

        return [functools.partial(piece, c) for c in range(0, 3 * D, 128)]

    def b_attn(buf, first_block):
        q_v, kv_v, ob_v = buf

        def shifted(w, r, c0):
            hi, j = divmod(w, 8 // _B_DIL)
            return kv_v[j, 8 - 8 * hi + r:8 - 8 * hi + r + _B_CHUNK, c0:c0 + D]

        def chunk(r):
            q = q_v[r:r + _B_CHUNK, :]
            part = []
            for w in range(_B_WIN):
                pr = q * shifted(w, r, 0)
                acc = pr[:, 0:128]
                for g in range(1, n_grp):
                    acc = acc + pr[:, g * 128:(g + 1) * 128]
                part.append(acc)
            full = _dot(jnp.concatenate(part, axis=0), _unpack(same_head_v[...])) * b_scale
            logits = []
            for w in range(_B_WIN):
                lg = full[w * _B_CHUNK:(w + 1) * _B_CHUNK]
                if first_block and r < w * _B_DIL:
                    pos = r + jax.lax.broadcasted_iota(jnp.int32, lg.shape, 0)
                    lg = jnp.where(pos >= w * _B_DIL, lg, -1e9)
                logits.append(lg)
            m = functools.reduce(jnp.maximum, logits)
            es = [jnp.exp(lg - m) for lg in logits]
            inv = 1.0 / functools.reduce(jnp.add, es)
            o = None
            for w in range(_B_WIN):
                t = jnp.concatenate([es[w] * inv] * n_grp, axis=1) * shifted(w, r, D)
                o = t if o is None else o + t
            ob_v[r // 2:(r + _B_CHUNK) // 2, :] = _pack(o.astype(BF16))

        return [functools.partial(chunk, r) for r in range(0, R, _B_CHUNK)]

    def b_out(i, buf):
        def piece(c):
            b_v[pl.ds(pl.multiple_of(i * R, R), R), c:c + 128] = _dot(
                _unpack(buf[2][...]), _unpack(bwop_v[:, c:c + 128]))

        return [functools.partial(piece, c) for c in range(0, D, 128)]

    def a_weights(i):
        def piece(t, c):
            if t < 3:
                w_v[i, :, t * pw + c:t * pw + c + 128] = _pack(wt_v[i, t, c:c + 128, :].T)
            else:
                wo_v[i, c // 2:c // 2 + 64, :] = _pack(wt_v[i, t, c:c + 128, :])

        return [functools.partial(piece, t, c) for t in range(4) for c in range(0, pw, 128)]

    a_scale = dh ** (-0.5)

    def tokens(s0, mem):
        xs = x_v[pl.ds(s0, seg), :].astype(F32)
        return xs, jnp.concatenate([xs, mem], axis=0)

    def block_diag(a):
        lo = jax.lax.broadcasted_iota(jnp.int32, (L, 128), 1) < (dh - 128)
        zero = jnp.zeros((L, 128), F32)
        mid = a[:, 128:256]
        top = jnp.concatenate([a[:, 0:128], jnp.where(lo, mid, 0.0), zero], axis=1)
        bot = jnp.concatenate([zero, jnp.where(lo, 0.0, mid), a[:, 256:384]], axis=1)
        return jnp.concatenate([top, bot], axis=0).astype(BF16)

    def a_proj(h, p):
        return _dot(h, _unpack(w_v[p]))

    def a_scores(qkv):
        sc = _dot(qkv[:, 0:pw], block_diag(qkv[:, pw:2 * pw]), _NT) * a_scale
        return sc, block_diag(qkv[:, 2 * pw:3 * pw])

    def a_softmax(sc):
        row = jax.lax.broadcasted_iota(jnp.int32, (L, 2 * L), 0)
        col = jax.lax.broadcasted_iota(jnp.int32, (L, 2 * L), 1)
        first = col < L
        key = jnp.where(first, col, col - L)
        sc = jnp.where((row >= seg) | (key >= seg) | (row >= key), sc, -1e9)
        m0 = jnp.max(jnp.where(first, sc, -jnp.inf), axis=1, keepdims=True)
        m1 = jnp.max(jnp.where(first, -jnp.inf, sc), axis=1, keepdims=True)
        e = jnp.exp(sc - jnp.where(first, m0, m1))
        l0 = jnp.sum(jnp.where(first, e, 0.0), axis=1, keepdims=True)
        l1 = jnp.sum(jnp.where(first, 0.0, e), axis=1, keepdims=True)
        return e / jnp.where(first, l0, l1)

    def a_out(o, p):
        return _dot(jnp.concatenate([o[seg:L], o[0:seg]], axis=0), _unpack(wo_v[p]))

    def mix(s0, xs, acc):
        g = jax.nn.sigmoid(jnp.sum(xs * gw_ref[...].astype(F32), axis=1, keepdims=True))
        res = g * acc[M:L] + (1.0 - g) * b_v[pl.ds(s0, seg), :]
        out_v[pl.ds(s0, seg), :] = res.astype(out_v.dtype)

    def first_segment(p):
        st = {}

        def proj():
            st[0] = a_proj(tokens(0, mem0_ref[...].astype(F32))[1], p)

        def scores():
            st[1] = a_scores(st[0])

        def values():
            st[2] = _dot(a_softmax(st[1][0]), st[1][1])

        def out():
            acc_v[...] += a_out(st[2], p)

        return [proj, scores, values, out]

    def startup(i, cur, oth, head=None, last=False):
        weights, seg0 = [], []
        if head is None or head >= 1:
            for t in range(4):
                cp_w(t, i - 1).wait()
            weights = a_weights(i - 1)
        if head is None:
            seg0 = first_segment(i - 2)
        mm = ([] if head == 0 else b_out(i - 1, oth)) + ([] if last else b_proj(i + 1, oth, cur))
        _interleave(mm, b_attn(cur, head == 0), weights, seg0)

    buf0, buf1 = (q0_v, kv0_v, ob0_v), (q1_v, kv1_v, ob1_v)
    acc_v[...] = jnp.zeros((L, D), F32)
    cp_x0.wait()
    _interleave(b_proj(0, buf0, None))
    cp_bwo.wait()
    for g in range(D // 128):
        tmp_v[g] = bwo_v[:, g * 128:(g + 1) * 128].astype(F32)
    permute_rows(bwop_v, 0)
    startup(0, buf0, buf1, head=0)
    cp_x1.wait()
    startup(1, buf1, buf0, head=1)

    def startup2(j, carry):
        startup(2 * j + 2, buf0, buf1)
        startup(2 * j + 3, buf1, buf0)
        return carry

    jax.lax.fori_loop(0, n_pairs // 2 - 2, startup2, 0)
    startup(n_pairs - 2, buf0, buf1)
    startup(n_pairs - 1, buf1, buf0, last=True)
    _interleave(b_out(n_pairs - 1, buf1), first_segment(n_pairs - 2))
    for t in range(4):
        cp_w(t, n_pairs - 1).wait()
    _interleave(a_weights(n_pairs - 1))
    _interleave(first_segment(n_pairs - 1))
    mix(0, tokens(0, mem0_ref[...].astype(F32))[0], acc_v[...])
    mem_v[...] = acc_v[0:M, :]
    pltpu.make_async_copy(out_v.at[pl.ds(0, seg)], out_hbm.at[pl.ds(0, seg)],
                          sem_out.at[0]).start()

    def step(s, mem):
        s0 = pl.multiple_of(s * seg, seg)
        xs, h = tokens(s0, mem)
        lag_s, lag_m, lag_v, lag_o = _LAGS
        qkv, sv, pr, o = {}, {}, {}, {}
        acc = None
        for i in range(n_pairs + lag_o):
            if i < n_pairs:
                qkv[i] = a_proj(h, i)
            if 0 <= i - lag_s < n_pairs:
                sv[i - lag_s] = a_scores(qkv.pop(i - lag_s))
            if 0 <= i - lag_m < n_pairs:
                pr[i - lag_m] = a_softmax(sv[i - lag_m][0])
            if 0 <= i - lag_v < n_pairs:
                o[i - lag_v] = _dot(pr.pop(i - lag_v), sv.pop(i - lag_v)[1])
            if 0 <= i - lag_o < n_pairs:
                t = a_out(o.pop(i - lag_o), i - lag_o)
                acc = t if acc is None else acc + t
        mix(s0, xs, acc)
        return acc[0:M]

    def steps(j, carry):
        mem = mem_v[...]
        for u in range(_UNROLL):
            mem = step(1 + j * _UNROLL + u, mem)
        mem_v[...] = mem
        rows = pl.ds(pl.multiple_of((1 + j * _UNROLL) * seg, seg), _UNROLL * seg)
        pltpu.make_async_copy(out_v.at[rows], out_hbm.at[rows], sem_out.at[0]).start()
        return carry

    jax.lax.fori_loop(0, (n_seg - 1) // _UNROLL, steps, 0)
    pltpu.make_async_copy(out_v, out_hbm, sem_out.at[0]).wait()


@functools.partial(jax.jit, static_argnames=("A_seg_len",))
def pallas_gated_mix__memory_aug_recurrent_mem_tr__sliding_local_dilated__prompt_kernel(
    A_x, A_mem0, A_Wq, A_Wk, A_Wv, A_Wo, A_seg_len, B_x, B_wqkv, B_wo, gate_w,
):
    del B_x
    _, S, D = A_x.shape
    M = A_mem0.shape[1]
    _, H, Dh = A_Wq.shape
    seg = int(A_seg_len)
    n_pairs = H // 2
    pw = 2 * Dh
    assert Dh == 192 and S == n_pairs * _B_ROWS and S % seg == 0 and D % 128 == 0
    assert (S // seg - 1) % _UNROLL == 0

    def wt(w):
        return jnp.transpose(w, (1, 2, 0)).reshape(n_pairs, pw, D)

    b_bufs = [pltpu.VMEM((_B_ROWS, D), F32),
              pltpu.VMEM((8 // _B_DIL, _B_ROWS + 8, 2 * D), F32),
              pltpu.VMEM((_B_ROWS // 2, D), U32)]
    hbm = pl.BlockSpec(memory_space=pl.ANY)
    vmem = pl.BlockSpec(memory_space=pltpu.VMEM)
    out = pl.pallas_call(
        functools.partial(_kernel, seg=seg, n_heads=H, dh=Dh),
        out_shape=jax.ShapeDtypeStruct((S, D), A_x.dtype),
        in_specs=[hbm, vmem, hbm, hbm, hbm, hbm, hbm, hbm, vmem],
        out_specs=hbm,
        scratch_shapes=[
            pltpu.VMEM((S, D), BF16),
            pltpu.VMEM((n_pairs, 4, pw, D), BF16),
            pltpu.VMEM((n_pairs, D // 2, 3 * pw), U32),
            pltpu.VMEM((n_pairs, pw // 2, D), U32),
            pltpu.VMEM((D, 3 * D), BF16),
            pltpu.VMEM((3 * D // 2, D), U32),
            pltpu.VMEM((D, D), BF16),
            pltpu.VMEM((D // 2, D), U32),
            pltpu.VMEM((D // 128, D, 128), F32),
            pltpu.VMEM((64, 128), U32),
            *b_bufs, *b_bufs,
            pltpu.VMEM((S, D), F32),
            pltpu.VMEM((M, D), F32),
            pltpu.VMEM((M + seg, D), F32),
            pltpu.VMEM((S, D), A_x.dtype),
            pltpu.SemaphoreType.DMA((4,)),
            pltpu.SemaphoreType.DMA((n_pairs, 4)),
            pltpu.SemaphoreType.DMA((1,)),
        ],
        compiler_params=pltpu.CompilerParams(vmem_limit_bytes=110 * 1024 * 1024),
    )(A_x.reshape(S, D), A_mem0.reshape(M, D), wt(A_Wq), wt(A_Wk), wt(A_Wv),
      A_Wo.reshape(n_pairs, pw, D), B_wqkv, B_wo, gate_w.reshape(1, D))
    return out.reshape(A_x.shape)
```

```python
import functools

import jax
import jax.numpy as jnp
import jax.experimental.pallas as pl
import jax.experimental.pallas.tpu as pltpu

F32 = jnp.float32
BF16 = jnp.bfloat16
U32 = jnp.uint32

_NN = (((1,), (0,)), ((), ()))
_NT = (((1,), (1,)), ((), ()))

_B_HEADS = 32
_B_WIN = 8
_B_DIL = 2
_B_PAD = 16
_B_CHUNK = 16
_B_ROWS = 128
_LAGS = (1, 2, 4, 6)
_UNROLL = 3


def _dot(a, b, dims=_NN):
    return jax.lax.dot_general(a, b, dims, preferred_element_type=F32)


def _pack(a):
    return pltpu.bitcast(a, U32)


def _unpack(a):
    return pltpu.bitcast(a, BF16)


def _interleave(*streams):
    todo = [((k + 0.5) / len(st), n, fn) for n, st in enumerate(streams) for k, fn in enumerate(st)]
    for _, _, fn in sorted(todo, key=lambda e: e[:2]):
        fn()


def _kernel(x_hbm, mem0_ref, wqt_hbm, wkt_hbm, wvt_hbm, wo_hbm, bwqkv_hbm,
            bwo_hbm, gw_ref, out_hbm,
            x_v, wt_v, w_v, wo_v, bw_v, bwp_v, bwo_v, bwop_v, tmp_v, same_head_v,
            q0_v, kv0_v, ob0_v, q1_v, kv1_v, ob1_v, b_v,
            mem_v, acc_v, out_v, sem_in, sem_w, sem_out, *, seg, n_heads, dh):
    S, D = x_v.shape
    M = mem0_ref.shape[0]
    L = M + seg
    n_seg = S // seg
    pw = 2 * dh
    n_pairs = n_heads // 2
    bdh = D // _B_HEADS

    cp_bw = pltpu.make_async_copy(bwqkv_hbm, bw_v, sem_in.at[0])
    x_head, x_tail = pl.ds(0, 2 * _B_ROWS), pl.ds(2 * _B_ROWS, S - 2 * _B_ROWS)
    cp_x0 = pltpu.make_async_copy(x_hbm.at[x_head], x_v.at[x_head], sem_in.at[1])
    cp_x1 = pltpu.make_async_copy(x_hbm.at[x_tail], x_v.at[x_tail], sem_in.at[3])
    cp_bwo = pltpu.make_async_copy(bwo_hbm, bwo_v, sem_in.at[2])

    def cp_w(t, p):
        src = (wqt_hbm, wkt_hbm, wvt_hbm, wo_hbm)[t]
        return pltpu.make_async_copy(src.at[p], wt_v.at[p, t], sem_w.at[p, t])

    cp_bw.start()
    cp_x0.start()
    cp_bwo.start()
    cp_x1.start()

    def permute_rows(dst_v, r0):
        for g in range(D // 128):
            for d in range(bdh):
                rows = tmp_v[g, pl.ds(d, _B_HEADS, stride=bdh), :]
                r = (r0 + d * _B_HEADS) // 2
                dst_v[r:r + _B_HEADS // 2, g * 128:(g + 1) * 128] = _pack(rows.astype(BF16))

    ri = jax.lax.broadcasted_iota(jnp.int32, (128, 128), 0)
    ci = jax.lax.broadcasted_iota(jnp.int32, (128, 128), 1)
    same_head_v[...] = _pack(jnp.where(ri % _B_HEADS == ci % _B_HEADS, 1.0, 0.0).astype(BF16))
    cp_bw.wait()
    for p in range(n_pairs):
        for t in range(4):
            cp_w(t, p).start()
    for t in range(3):
        for g in range(D // 128):
            tmp_v[g] = bw_v[g * 128:(g + 1) * 128, t * D:(t + 1) * D].T.astype(F32)
        permute_rows(bwp_v, t * D)

    b_scale = bdh ** (-0.5)
    n_grp = D // 128
    R, P = _B_ROWS, _B_PAD

    def b_proj(i, buf, prev):
        q_v, kv_v, _ = buf
        xb = x_v[pl.ds(pl.multiple_of(i * R, R), R), :]

        def piece(c):
            y = _dot(xb, _unpack(bwp_v[c // 2:c // 2 + 64, :]), _NT)
            if c < D:
                q_v[:, c:c + 128] = y
                return
            cols = slice(c - D, c - D + 128)
            halo = jnp.zeros((P, 128), F32) if prev is None else prev[1][0, R - 8:R + 8, cols]
            y = jnp.concatenate([halo, y], axis=0)
            for j in range(8 // _B_DIL):
                kv_v[j, :, cols] = y[P - 8 - j * _B_DIL:P + R - j * _B_DIL]

        return [functools.partial(piece, c) for c in range(0, 3 * D, 128)]

    def b_attn(buf, first_block):
        q_v, kv_v, ob_v = buf

        def shifted(w, r, c0):
            hi, j = divmod(w, 8 // _B_DIL)
            return kv_v[j, 8 - 8 * hi + r:8 - 8 * hi + r + _B_CHUNK, c0:c0 + D]

        def chunk(r):
            q = q_v[r:r + _B_CHUNK, :]
            part = []
            for w in range(_B_WIN):
                pr = q * shifted(w, r, 0)
                acc = pr[:, 0:128]
                for g in range(1, n_grp):
                    acc = acc + pr[:, g * 128:(g + 1) * 128]
                part.append(acc)
            full = _dot(jnp.concatenate(part, axis=0), _unpack(same_head_v[...])) * b_scale
            logits = []
            for w in range(_B_WIN):
                lg = full[w * _B_CHUNK:(w + 1) * _B_CHUNK]
                if first_block and r < w * _B_DIL:
                    pos = r + jax.lax.broadcasted_iota(jnp.int32, lg.shape, 0)
                    lg = jnp.where(pos >= w * _B_DIL, lg, -1e9)
                logits.append(lg)
            m = functools.reduce(jnp.maximum, logits)
            es = [jnp.exp(lg - m) for lg in logits]
            inv = 1.0 / functools.reduce(jnp.add, es)
            o = None
            for w in range(_B_WIN):
                t = jnp.concatenate([es[w] * inv] * n_grp, axis=1) * shifted(w, r, D)
                o = t if o is None else o + t
            ob_v[r // 2:(r + _B_CHUNK) // 2, :] = _pack(o.astype(BF16))

        return [functools.partial(chunk, r) for r in range(0, R, _B_CHUNK)]

    def b_out(i, buf):
        def piece(c):
            b_v[pl.ds(pl.multiple_of(i * R, R), R), c:c + 128] = _dot(
                _unpack(buf[2][...]), _unpack(bwop_v[:, c:c + 128]))

        return [functools.partial(piece, c) for c in range(0, D, 128)]

    def a_weights(i):
        def piece(t, c):
            if t < 3:
                w_v[i, :, t * pw + c:t * pw + c + 128] = _pack(wt_v[i, t, c:c + 128, :].T)
            else:
                wo_v[i, c // 2:c // 2 + 64, :] = _pack(wt_v[i, t, c:c + 128, :])

        return [functools.partial(piece, t, c) for t in range(4) for c in range(0, pw, 128)]

    a_scale = dh ** (-0.5)

    def tokens(s0, mem):
        xs = x_v[pl.ds(s0, seg), :].astype(F32)
        return xs, jnp.concatenate([xs, mem], axis=0)

    def block_diag(a):
        lo = jax.lax.broadcasted_iota(jnp.int32, (L, 128), 1) < (dh - 128)
        zero = jnp.zeros((L, 128), F32)
        mid = a[:, 128:256]
        top = jnp.concatenate([a[:, 0:128], jnp.where(lo, mid, 0.0), zero], axis=1)
        bot = jnp.concatenate([zero, jnp.where(lo, 0.0, mid), a[:, 256:384]], axis=1)
        return jnp.concatenate([top, bot], axis=0).astype(BF16)

    def a_proj(h, p):
        return _dot(h, _unpack(w_v[p]))

    def a_scores(qkv):
        sc = _dot(qkv[:, 0:pw], block_diag(qkv[:, pw:2 * pw]), _NT) * a_scale
        return sc, block_diag(qkv[:, 2 * pw:3 * pw])

    def a_softmax(sc):
        row = jax.lax.broadcasted_iota(jnp.int32, (L, 2 * L), 0)
        col = jax.lax.broadcasted_iota(jnp.int32, (L, 2 * L), 1)
        first = col < L
        key = jnp.where(first, col, col - L)
        sc = jnp.where((row >= seg) | (key >= seg) | (row >= key), sc, -1e9)
        m0 = jnp.max(jnp.where(first, sc, -jnp.inf), axis=1, keepdims=True)
        m1 = jnp.max(jnp.where(first, -jnp.inf, sc), axis=1, keepdims=True)
        e = jnp.exp(sc - jnp.where(first, m0, m1))
        l0 = jnp.sum(jnp.where(first, e, 0.0), axis=1, keepdims=True)
        l1 = jnp.sum(jnp.where(first, 0.0, e), axis=1, keepdims=True)
        return e / jnp.where(first, l0, l1)

    def a_out(o, p):
        return _dot(jnp.concatenate([o[seg:L], o[0:seg]], axis=0), _unpack(wo_v[p]))

    def mix(s0, xs, acc):
        g = jax.nn.sigmoid(jnp.sum(xs * gw_ref[...].astype(F32).reshape(1, D), axis=1, keepdims=True))
        res = g * acc[M:L] + (1.0 - g) * b_v[pl.ds(s0, seg), :]
        out_v[pl.ds(s0, seg), :] = res.astype(out_v.dtype)

    def first_segment(p):
        st = {}

        def proj():
            st[0] = a_proj(tokens(0, mem0_ref[...].astype(F32))[1], p)

        def scores():
            st[1] = a_scores(st[0])

        def values():
            st[2] = _dot(a_softmax(st[1][0]), st[1][1])

        def out():
            acc_v[...] += a_out(st[2], p)

        return [proj, scores, values, out]

    def startup(i, cur, oth, head=None, last=False):
        weights, seg0 = [], []
        if head is None or head >= 1:
            for t in range(4):
                cp_w(t, i - 1).wait()
            weights = a_weights(i - 1)
        if last:
            for t in range(4):
                cp_w(t, i).wait()
            weights = weights + a_weights(i)
        if head is None:
            seg0 = first_segment(i - 2)
        mm = ([] if head == 0 else b_out(i - 1, oth)) + ([] if last else b_proj(i + 1, oth, cur))
        _interleave(mm, b_attn(cur, head == 0), weights, seg0)

    buf0, buf1 = (q0_v, kv0_v, ob0_v), (q1_v, kv1_v, ob1_v)
    acc_v[...] = jnp.zeros((L, D), F32)
    cp_x0.wait()
    _interleave(b_proj(0, buf0, None))
    cp_bwo.wait()
    for g in range(D // 128):
        tmp_v[g] = bwo_v[:, g * 128:(g + 1) * 128].astype(F32)
    permute_rows(bwop_v, 0)
    startup(0, buf0, buf1, head=0)
    cp_x1.wait()
    startup(1, buf1, buf0, head=1)

    def startup2(j, carry):
        startup(2 * j + 2, buf0, buf1)
        startup(2 * j + 3, buf1, buf0)
        return carry

    jax.lax.fori_loop(0, n_pairs // 2 - 2, startup2, 0)
    startup(n_pairs - 2, buf0, buf1)
    startup(n_pairs - 1, buf1, buf0, last=True)
    _interleave(first_segment(n_pairs - 2), first_segment(n_pairs - 1), b_out(n_pairs - 1, buf1))
    mix(0, tokens(0, mem0_ref[...].astype(F32))[0], acc_v[...])
    mem_v[...] = acc_v[0:M, :]
    pltpu.make_async_copy(out_v.at[pl.ds(0, seg)], out_hbm.at[pl.ds(0, seg)],
                          sem_out.at[0]).start()

    def step(s, mem):
        s0 = pl.multiple_of(s * seg, seg)
        xs, h = tokens(s0, mem)
        lag_s, lag_m, lag_v, lag_o = _LAGS
        qkv, sv, pr, o = {}, {}, {}, {}
        acc = None
        for i in range(n_pairs + lag_o):
            if i < n_pairs:
                qkv[i] = a_proj(h, i)
            if 0 <= i - lag_s < n_pairs:
                sv[i - lag_s] = a_scores(qkv.pop(i - lag_s))
            if 0 <= i - lag_m < n_pairs:
                pr[i - lag_m] = a_softmax(sv[i - lag_m][0])
            if 0 <= i - lag_v < n_pairs:
                o[i - lag_v] = _dot(pr.pop(i - lag_v), sv.pop(i - lag_v)[1])
            if 0 <= i - lag_o < n_pairs:
                t = a_out(o.pop(i - lag_o), i - lag_o)
                acc = t if acc is None else acc + t
        mix(s0, xs, acc)
        return acc[0:M]

    def steps(j, carry):
        mem = mem_v[...]
        for u in range(_UNROLL):
            mem = step(1 + j * _UNROLL + u, mem)
        mem_v[...] = mem
        rows = pl.ds(pl.multiple_of((1 + j * _UNROLL) * seg, seg), _UNROLL * seg)
        pltpu.make_async_copy(out_v.at[rows], out_hbm.at[rows], sem_out.at[0]).start()
        return carry

    jax.lax.fori_loop(0, (n_seg - 1) // _UNROLL, steps, 0)
    pltpu.make_async_copy(out_v, out_hbm, sem_out.at[0]).wait()


@functools.partial(jax.jit, static_argnames=("A_seg_len",))
def pallas_gated_mix__memory_aug_recurrent_mem_tr__sliding_local_dilated__prompt_kernel(
    A_x, A_mem0, A_Wq, A_Wk, A_Wv, A_Wo, A_seg_len, B_x, B_wqkv, B_wo, gate_w,
):
    del B_x
    _, S, D = A_x.shape
    M = A_mem0.shape[1]
    _, H, Dh = A_Wq.shape
    seg = int(A_seg_len)
    n_pairs = H // 2
    pw = 2 * Dh
    assert Dh == 192 and S == n_pairs * _B_ROWS and S % seg == 0 and D % 128 == 0
    assert (S // seg - 1) % _UNROLL == 0

    def wt(w):
        return jnp.transpose(w, (1, 2, 0)).reshape(n_pairs, pw, D)

    b_bufs = [pltpu.VMEM((_B_ROWS, D), F32),
              pltpu.VMEM((8 // _B_DIL, _B_ROWS + 8, 2 * D), F32),
              pltpu.VMEM((_B_ROWS // 2, D), U32)]
    hbm = pl.BlockSpec(memory_space=pl.ANY)
    vmem = pl.BlockSpec(memory_space=pltpu.VMEM)
    out = pl.pallas_call(
        functools.partial(_kernel, seg=seg, n_heads=H, dh=Dh),
        out_shape=jax.ShapeDtypeStruct((S, D), A_x.dtype),
        in_specs=[hbm, vmem, hbm, hbm, hbm, hbm, hbm, hbm, vmem],
        out_specs=hbm,
        scratch_shapes=[
            pltpu.VMEM((S, D), BF16),
            pltpu.VMEM((n_pairs, 4, pw, D), BF16),
            pltpu.VMEM((n_pairs, D // 2, 3 * pw), U32),
            pltpu.VMEM((n_pairs, pw // 2, D), U32),
            pltpu.VMEM((D, 3 * D), BF16),
            pltpu.VMEM((3 * D // 2, D), U32),
            pltpu.VMEM((D, D), BF16),
            pltpu.VMEM((D // 2, D), U32),
            pltpu.VMEM((D // 128, D, 128), F32),
            pltpu.VMEM((64, 128), U32),
            *b_bufs, *b_bufs,
            pltpu.VMEM((S, D), F32),
            pltpu.VMEM((M, D), F32),
            pltpu.VMEM((M + seg, D), F32),
            pltpu.VMEM((S, D), A_x.dtype),
            pltpu.SemaphoreType.DMA((4,)),
            pltpu.SemaphoreType.DMA((n_pairs, 4)),
            pltpu.SemaphoreType.DMA((1,)),
        ],
        compiler_params=pltpu.CompilerParams(vmem_limit_bytes=110 * 1024 * 1024),
    )(A_x.reshape(S, D), A_mem0.reshape(M, D), wt(A_Wq), wt(A_Wk), wt(A_Wv),
      A_Wo.reshape(n_pairs, pw, D), B_wqkv, B_wo, gate_w)
    return out.reshape(A_x.shape)
```

```python
import functools

import jax
import jax.numpy as jnp
import jax.experimental.pallas as pl
import jax.experimental.pallas.tpu as pltpu

F32 = jnp.float32
BF16 = jnp.bfloat16
U32 = jnp.uint32

_NN = (((1,), (0,)), ((), ()))
_NT = (((1,), (1,)), ((), ()))

_B_HEADS = 32
_B_WIN = 8
_B_DIL = 2
_B_PAD = 16
_B_CHUNK = 16
_B_ROWS = 128
_LAGS = (1, 2, 4, 6)
_UNROLL = 3


def _dot(a, b, dims=_NN):
    return jax.lax.dot_general(a, b, dims, preferred_element_type=F32)


def _pack(a):
    return pltpu.bitcast(a, U32)


def _unpack(a):
    return pltpu.bitcast(a, BF16)


def _interleave(*streams):
    todo = [((k + 0.5) / len(st), n, fn) for n, st in enumerate(streams) for k, fn in enumerate(st)]
    for _, _, fn in sorted(todo, key=lambda e: e[:2]):
        fn()


def _kernel(x_hbm, mem0_hbm, wqt_hbm, wkt_hbm, wvt_hbm, wo_hbm, bwqkv_hbm,
            bwo_hbm, gw_hbm, out_hbm,
            x_v, wt_v, w_v, wo_v, bw_v, bwp_v, bwo_v, bwop_v, tmp_v, same_head_v,
            q0_v, kv0_v, ob0_v, q1_v, kv1_v, ob1_v, b_v,
            mem0_v, gw_v, mem_v, acc_v, out_v, sem_in, sem_w, sem_out, *, seg, n_heads, dh):
    S, D = x_v.shape
    M = mem0_v.shape[0]
    L = M + seg
    n_seg = S // seg
    pw = 2 * dh
    n_pairs = n_heads // 2
    bdh = D // _B_HEADS

    n_grp = D // 128
    x_head, x_tail = pl.ds(0, 2 * _B_ROWS), pl.ds(2 * _B_ROWS, S - 2 * _B_ROWS)
    cp_x0 = pltpu.make_async_copy(x_hbm.at[x_head], x_v.at[x_head], sem_in.at[0])
    cp_x1 = pltpu.make_async_copy(x_hbm.at[x_tail], x_v.at[x_tail], sem_in.at[1])
    cp_bwo = pltpu.make_async_copy(bwo_hbm, bwo_v, sem_in.at[2])
    cp_mem0 = pltpu.make_async_copy(mem0_hbm, mem0_v, sem_in.at[3])
    cp_gw = pltpu.make_async_copy(gw_hbm, gw_v, sem_in.at[4])

    def cp_bw(g):
        rows = pl.ds(g * 128, 128)
        return pltpu.make_async_copy(bwqkv_hbm.at[rows], bw_v.at[rows], sem_in.at[5 + g])

    def cp_w(t, p):
        src = (wqt_hbm, wkt_hbm, wvt_hbm, wo_hbm)[t]
        return pltpu.make_async_copy(src.at[p], wt_v.at[p, t], sem_w.at[p, t])

    for g in range(n_grp):
        cp_bw(g).start()
    for cp in (cp_x0, cp_bwo, cp_mem0, cp_gw):
        cp.start()

    def permute_rows(dst_v, r0, g, a):
        tmp_v[0:D, :] = a.astype(F32)
        for d in range(bdh):
            rows = tmp_v[pl.ds(d, _B_HEADS, stride=bdh), :]
            r = (r0 + d * _B_HEADS) // 2
            dst_v[r:r + _B_HEADS // 2, g * 128:(g + 1) * 128] = _pack(rows.astype(BF16))

    ri = jax.lax.broadcasted_iota(jnp.int32, (128, 128), 0)
    ci = jax.lax.broadcasted_iota(jnp.int32, (128, 128), 1)
    same_head_v[...] = _pack(jnp.where(ri % _B_HEADS == ci % _B_HEADS, 1.0, 0.0).astype(BF16))
    for g in range(n_grp):
        cp_bw(g).wait()
        if g == 0:
            cp_x1.start()
        if g == n_grp - 1:
            for p in range(n_pairs):
                for t in range(4):
                    cp_w(t, p).start()
        for t in range(3):
            permute_rows(bwp_v, t * D, g, bw_v[g * 128:(g + 1) * 128, t * D:(t + 1) * D].T)

    b_scale = bdh ** (-0.5)
    R, P = _B_ROWS, _B_PAD

    def b_proj(i, buf, prev):
        q_v, kv_v, _ = buf
        xb = x_v[pl.ds(pl.multiple_of(i * R, R), R), :]

        def piece(c):
            y = _dot(xb, _unpack(bwp_v[c // 2:c // 2 + 64, :]), _NT)
            if c < D:
                q_v[:, c:c + 128] = y
                return
            cols = slice(c - D, c - D + 128)
            halo = jnp.zeros((P, 128), F32) if prev is None else prev[1][0, R - 8:R + 8, cols]
            y = jnp.concatenate([halo, y], axis=0)
            for j in range(8 // _B_DIL):
                kv_v[j, :, cols] = y[P - 8 - j * _B_DIL:P + R - j * _B_DIL]

        return [functools.partial(piece, c) for c in range(0, 3 * D, 128)]

    def b_attn(buf, first_block):
        q_v, kv_v, ob_v = buf

        def shifted(w, r, c0):
            hi, j = divmod(w, 8 // _B_DIL)
            return kv_v[j, 8 - 8 * hi + r:8 - 8 * hi + r + _B_CHUNK, c0:c0 + D]

        def chunk(r):
            q = q_v[r:r + _B_CHUNK, :]
            part = []
            for w in range(_B_WIN):
                pr = q * shifted(w, r, 0)
                acc = pr[:, 0:128]
                for g in range(1, n_grp):
                    acc = acc + pr[:, g * 128:(g + 1) * 128]
                part.append(acc)
            full = _dot(jnp.concatenate(part, axis=0), _unpack(same_head_v[...])) * b_scale
            logits = []
            for w in range(_B_WIN):
                lg = full[w * _B_CHUNK:(w + 1) * _B_CHUNK]
                if first_block and r < w * _B_DIL:
                    pos = r + jax.lax.broadcasted_iota(jnp.int32, lg.shape, 0)
                    lg = jnp.where(pos >= w * _B_DIL, lg, -1e9)
                logits.append(lg)
            m = functools.reduce(jnp.maximum, logits)
            es = [jnp.exp(lg - m) for lg in logits]
            inv = 1.0 / functools.reduce(jnp.add, es)
            o = None
            for w in range(_B_WIN):
                t = jnp.concatenate([es[w] * inv] * n_grp, axis=1) * shifted(w, r, D)
                o = t if o is None else o + t
            ob_v[r // 2:(r + _B_CHUNK) // 2, :] = _pack(o.astype(BF16))

        return [functools.partial(chunk, r) for r in range(0, R, _B_CHUNK)]

    def b_out(i, buf):
        def piece(c):
            b_v[pl.ds(pl.multiple_of(i * R, R), R), c:c + 128] = _dot(
                _unpack(buf[2][...]), _unpack(bwop_v[:, c:c + 128]))

        return [functools.partial(piece, c) for c in range(0, D, 128)]

    def a_weights(i):
        def piece(t, c):
            if t < 3:
                w_v[i, :, t * pw + c:t * pw + c + 128] = _pack(wt_v[i, t, c:c + 128, :].T)
            else:
                wo_v[i, c // 2:c // 2 + 64, :] = _pack(wt_v[i, t, c:c + 128, :])

        return [functools.partial(piece, t, c) for t in range(4) for c in range(0, pw, 128)]

    a_scale = dh ** (-0.5)

    def tokens(s0, mem):
        xs = x_v[pl.ds(s0, seg), :].astype(F32)
        return xs, jnp.concatenate([xs, mem], axis=0)

    def block_diag(a):
        lo = jax.lax.broadcasted_iota(jnp.int32, (L, 128), 1) < (dh - 128)
        zero = jnp.zeros((L, 128), F32)
        mid = a[:, 128:256]
        top = jnp.concatenate([a[:, 0:128], jnp.where(lo, mid, 0.0), zero], axis=1)
        bot = jnp.concatenate([zero, jnp.where(lo, 0.0, mid), a[:, 256:384]], axis=1)
        return jnp.concatenate([top, bot], axis=0).astype(BF16)

    def a_proj(h, p):
        return _dot(h, _unpack(w_v[p]))

    def a_scores(qkv):
        sc = _dot(qkv[:, 0:pw], block_diag(qkv[:, pw:2 * pw]), _NT) * a_scale
        return sc, block_diag(qkv[:, 2 * pw:3 * pw])

    def a_softmax(sc):
        row = jax.lax.broadcasted_iota(jnp.int32, (L, 2 * L), 0)
        col = jax.lax.broadcasted_iota(jnp.int32, (L, 2 * L), 1)
        first = col < L
        key = jnp.where(first, col, col - L)
        sc = jnp.where((row >= seg) | (key >= seg) | (row >= key), sc, -1e9)
        m0 = jnp.max(jnp.where(first, sc, -jnp.inf), axis=1, keepdims=True)
        m1 = jnp.max(jnp.where(first, -jnp.inf, sc), axis=1, keepdims=True)
        e = jnp.exp(sc - jnp.where(first, m0, m1))
        l0 = jnp.sum(jnp.where(first, e, 0.0), axis=1, keepdims=True)
        l1 = jnp.sum(jnp.where(first, 0.0, e), axis=1, keepdims=True)
        return e / jnp.where(first, l0, l1)

    def a_out(o, p):
        return _dot(jnp.concatenate([o[seg:L], o[0:seg]], axis=0), _unpack(wo_v[p]))

    def mix(s0, xs, acc):
        g = jax.nn.sigmoid(jnp.sum(xs * gw_v[...].astype(F32).reshape(1, D), axis=1, keepdims=True))
        res = g * acc[M:L] + (1.0 - g) * b_v[pl.ds(s0, seg), :]
        out_v[pl.ds(s0, seg), :] = res.astype(out_v.dtype)

    def first_segment(p):
        st = {}

        def proj():
            st[0] = a_proj(tokens(0, mem0_v[...].astype(F32))[1], p)

        def scores():
            st[1] = a_scores(st[0])

        def values():
            st[2] = _dot(a_softmax(st[1][0]), st[1][1])

        def out():
            acc_v[...] += a_out(st[2], p)

        return [proj, scores, values, out]

    def startup(i, cur, oth, head=None, last=False):
        weights, seg0 = [], []
        if head is None or head >= 1:
            for t in range(4):
                cp_w(t, i - 1).wait()
            weights = a_weights(i - 1)
        if last:
            for t in range(4):
                cp_w(t, i).wait()
            weights = weights + a_weights(i)
        if head is None:
            seg0 = first_segment(i - 2)
        mm = ([] if head == 0 else b_out(i - 1, oth)) + ([] if last else b_proj(i + 1, oth, cur))
        _interleave(mm, b_attn(cur, head == 0), weights, seg0)

    buf0, buf1 = (q0_v, kv0_v, ob0_v), (q1_v, kv1_v, ob1_v)
    acc_v[...] = jnp.zeros((L, D), F32)
    cp_x0.wait()
    _interleave(b_proj(0, buf0, None))
    cp_bwo.wait()
    for g in range(n_grp):
        permute_rows(bwop_v, 0, g, bwo_v[:, g * 128:(g + 1) * 128])
    startup(0, buf0, buf1, head=0)
    cp_mem0.wait()
    cp_gw.wait()
    cp_x1.wait()
    startup(1, buf1, buf0, head=1)

    def startup2(j, carry):
        startup(2 * j + 2, buf0, buf1)
        startup(2 * j + 3, buf1, buf0)
        return carry

    jax.lax.fori_loop(0, n_pairs // 2 - 2, startup2, 0)
    startup(n_pairs - 2, buf0, buf1)
    startup(n_pairs - 1, buf1, buf0, last=True)
    _interleave(first_segment(n_pairs - 2), first_segment(n_pairs - 1), b_out(n_pairs - 1, buf1))
    mix(0, tokens(0, mem0_v[...].astype(F32))[0], acc_v[...])
    mem_v[...] = acc_v[0:M, :]
    pltpu.make_async_copy(out_v.at[pl.ds(0, seg)], out_hbm.at[pl.ds(0, seg)],
                          sem_out.at[0]).start()

    def step(s, mem):
        s0 = pl.multiple_of(s * seg, seg)
        xs, h = tokens(s0, mem)
        lag_s, lag_m, lag_v, lag_o = _LAGS
        qkv, sv, pr, o = {}, {}, {}, {}
        acc = None
        for i in range(n_pairs + lag_o):
            if i < n_pairs:
                qkv[i] = a_proj(h, i)
            if 0 <= i - lag_s < n_pairs:
                sv[i - lag_s] = a_scores(qkv.pop(i - lag_s))
            if 0 <= i - lag_m < n_pairs:
                pr[i - lag_m] = a_softmax(sv[i - lag_m][0])
            if 0 <= i - lag_v < n_pairs:
                o[i - lag_v] = _dot(pr.pop(i - lag_v), sv.pop(i - lag_v)[1])
            if 0 <= i - lag_o < n_pairs:
                t = a_out(o.pop(i - lag_o), i - lag_o)
                acc = t if acc is None else acc + t
        mix(s0, xs, acc)
        return acc[0:M]

    def steps(j, carry):
        mem = mem_v[...]
        for u in range(_UNROLL):
            mem = step(1 + j * _UNROLL + u, mem)
        mem_v[...] = mem
        rows = pl.ds(pl.multiple_of((1 + j * _UNROLL) * seg, seg), _UNROLL * seg)
        pltpu.make_async_copy(out_v.at[rows], out_hbm.at[rows], sem_out.at[0]).start()
        return carry

    jax.lax.fori_loop(0, (n_seg - 1) // _UNROLL, steps, 0)
    pltpu.make_async_copy(out_v, out_hbm, sem_out.at[0]).wait()


@functools.partial(jax.jit, static_argnames=("A_seg_len",))
def pallas_gated_mix__memory_aug_recurrent_mem_tr__sliding_local_dilated__prompt_kernel(
    A_x, A_mem0, A_Wq, A_Wk, A_Wv, A_Wo, A_seg_len, B_x, B_wqkv, B_wo, gate_w,
):
    del B_x
    _, S, D = A_x.shape
    M = A_mem0.shape[1]
    _, H, Dh = A_Wq.shape
    seg = int(A_seg_len)
    n_pairs = H // 2
    pw = 2 * Dh
    assert Dh == 192 and S == n_pairs * _B_ROWS and S % seg == 0 and D % 128 == 0
    assert (S // seg - 1) % _UNROLL == 0

    def wt(w):
        return jnp.transpose(w, (1, 2, 0)).reshape(n_pairs, pw, D)

    b_bufs = [pltpu.VMEM((_B_ROWS, D), F32),
              pltpu.VMEM((8 // _B_DIL, _B_ROWS + 8, 2 * D), F32),
              pltpu.VMEM((_B_ROWS // 2, D), U32)]
    hbm = pl.BlockSpec(memory_space=pl.ANY)
    out = pl.pallas_call(
        functools.partial(_kernel, seg=seg, n_heads=H, dh=Dh),
        out_shape=jax.ShapeDtypeStruct((S, D), A_x.dtype),
        in_specs=[hbm] * 9,
        out_specs=hbm,
        scratch_shapes=[
            pltpu.VMEM((S, D), BF16),
            pltpu.VMEM((n_pairs, 4, pw, D), BF16),
            pltpu.VMEM((n_pairs, D // 2, 3 * pw), U32),
            pltpu.VMEM((n_pairs, pw // 2, D), U32),
            pltpu.VMEM((D, 3 * D), BF16),
            pltpu.VMEM((3 * D // 2, D), U32),
            pltpu.VMEM((D, D), BF16),
            pltpu.VMEM((D // 2, D), U32),
            pltpu.VMEM((D + 32, 128), F32),
            pltpu.VMEM((64, 128), U32),
            *b_bufs, *b_bufs,
            pltpu.VMEM((S, D), F32),
            pltpu.VMEM((M, D), A_mem0.dtype),
            pltpu.VMEM((D,), gate_w.dtype),
            pltpu.VMEM((M, D), F32),
            pltpu.VMEM((M + seg, D), F32),
            pltpu.VMEM((S, D), A_x.dtype),
            pltpu.SemaphoreType.DMA((5 + D // 128,)),
            pltpu.SemaphoreType.DMA((n_pairs, 4)),
            pltpu.SemaphoreType.DMA((1,)),
        ],
        compiler_params=pltpu.CompilerParams(vmem_limit_bytes=110 * 1024 * 1024),
    )(A_x.reshape(S, D), A_mem0.reshape(M, D), wt(A_Wq), wt(A_Wk), wt(A_Wv),
      A_Wo.reshape(n_pairs, pw, D), B_wqkv, B_wo, gate_w)
    return out.reshape(A_x.shape)
```
